```python
import os as _os
_os.environ.setdefault("JAX_PLATFORMS", "cpu")
import jax
import jax.numpy as jnp

def _softmax(x, axis=-1):
    return jax.nn.softmax(x, axis=axis)
def _gelu(x):
    return jax.nn.gelu(x, approximate=True)
def _silu(x):
    return jax.nn.silu(x)
def _sigmoid(x):
    return jax.nn.sigmoid(x)
def _layernorm(x, axis=-1, eps=1e-5):
    m = jnp.mean(x, axis=axis, keepdims=True)
    v = jnp.var(x, axis=axis, keepdims=True)
    return (x - m) / jnp.sqrt(v + eps)
def _scatter_add(tgt, idx, src, axis=0):
    return tgt.at[idx].add(src)
def _segment_sum(src, seg, n):
    return jax.ops.segment_sum(src, seg, n)
class _Rng:
    def __init__(self, key):
        self._k = key
    def _next(self):
        self._k, sub = jax.random.split(self._k)
        return sub
    def normal(self, shape):
        return jax.random.normal(self._next(), shape, dtype=jnp.bfloat16)
    def randint(self, lo, hi, shape):
        return jax.random.randint(self._next(), shape, lo, hi, dtype=jnp.int32)
    def uniform(self, shape, lo=0.0, hi=1.0):
        return jax.random.uniform(self._next(), shape, jnp.bfloat16, lo, hi)
    def permutation(self, n):
        return jax.random.permutation(self._next(), n)


kernel_name = 'interleave_layers__linear_attn_block__mha_block__prompt'

def setup_inputs():
    _rng = _Rng(jax.random.key(int.from_bytes(__import__("os").urandom(4), "little")))
    _w = (lambda a: (lambda t: t.astype(jnp.bfloat16) if jnp.issubdtype(t.dtype, jnp.floating) else t)(jnp.asarray(a)))
    def _A_setup():
        B, S, D = 1, 2048, 1024
        return {
            "x": _w((lambda *s: _rng.normal(s) * 0.05)(B, S, D)),
            "wqkv": _w((lambda *s: _rng.normal(s) * 0.1)(D, 3 * D)),
            "wo": _w((lambda *s: _rng.normal(s) * 0.1)(D, D)),
        }
    _A_in = _A_setup()

    def _B_setup():
        B, S, D, H = 1, 2048, 1024, 32
        return {
            "x": _w((lambda *s: _rng.normal(s) * 0.05)(B, S, D)),
            "wqkv": _w((lambda *s: _rng.normal(s) * 0.1)(D, 3 * D)),
            "wo": _w((lambda *s: _rng.normal(s) * 0.05)(D, D)),
        }
    _B_in = _B_setup()

    return {
        "A_x": _A_in["x"],
        "A_wqkv": _A_in["wqkv"],
        "A_wo": _A_in["wo"],
        "B_x": _B_in["x"],
        "B_wqkv": _B_in["wqkv"],
        "B_wo": _B_in["wo"],
    }

def reference(A_x, A_wqkv, A_wo, B_x, B_wqkv, B_wo):
    def _A_ref(x, wqkv, wo):
        B, S, D = x.shape
        H = 32; Dh = D // H
        qkv = (lambda x, *d: x.transpose(*d))((x @ wqkv).reshape(B, S, 3, H, Dh), 2, 0, 3, 1, 4)
        q, k, v = qkv[0], qkv[1], qkv[2]
        phi = lambda t: jnp.where(t > 0, t + 1, jnp.exp(t)) + 1e-6
        pq, pk = phi(q), phi(k)
        kv = jnp.einsum("bhsd,bhse->bhde", pk, v)
        z = jnp.einsum("bhsd->bhd", pk)
        num = jnp.einsum("bhqd,bhde->bhqe", pq, kv)
        den = jnp.einsum("bhqd,bhd->bhq", pq, z)[..., None] + 1e-6
        o = num / den
        return (lambda x, *d: x.transpose(*d))(o, 0, 2, 1, 3).reshape(B, S, D) @ wo

    def _B_ref(x, wqkv, wo):
        B, S, D = x.shape
        H = 32
        Dh = D // H
        qkv = (lambda x, *d: x.transpose(*d))((x @ wqkv).reshape(B, S, 3, H, Dh), 2, 0, 3, 1, 4)
        q, k, v = qkv[0], qkv[1], qkv[2]
        scores = jnp.einsum("bhqd,bhkd->bhqk", q, k) * (Dh ** -0.5)
        p = _softmax(scores, axis=-1)
        o = jnp.einsum("bhqk,bhkd->bhqd", p, v)
        return (lambda x, *d: x.transpose(*d))(o, 0, 2, 1, 3).reshape(B, S, D) @ wo

    x = A_x
    x = x + _A_ref(_layernorm(x, axis=-1), A_wqkv, A_wo)
    x = x + _B_ref(_layernorm(x, axis=-1), B_wqkv, B_wo)
    x = x + _A_ref(_layernorm(x, axis=-1), A_wqkv, A_wo)
    x = x + _B_ref(_layernorm(x, axis=-1), B_wqkv, B_wo)
    return x
```

```python
import functools
import math

import jax
import jax.numpy as jnp
from jax import lax
import jax.experimental.pallas as pl
import jax.experimental.pallas.tpu as pltpu

S = 2048
D = 1024
H = 32
DH = D // H
G = D // 128
HPG = 128 // DH
TM = 256
NTM = S // TM
TQ = 512
TK = 128
NQ = S // TQ
NC = S // TK

F32 = jnp.float32
BF16 = jnp.bfloat16
NT_DIMS = (((1,), (1,)), ((), ()))
QSCALE = (DH ** -0.5) * math.log2(math.e)


def _layernorm(x):
    m = jnp.mean(x, axis=-1, keepdims=True)
    xc = x - m
    v = jnp.mean(xc * xc, axis=-1, keepdims=True)
    return xc * lax.rsqrt(v + 1e-5)


def _phi(t):
    return jnp.where(t > 0, t + 1.0, jnp.exp(t)) + 1e-6


def _mm(a, b):
    return jnp.dot(a, b, preferred_element_type=F32)


def _kernel(x_hbm, wa_qkv_hbm, wa_o_hbm, wb_qkv_hbm, wb_o_hbm, out_hbm,
            xio_s, x_s, wa_qkv, wa_o, wb_qkv, wb_o,
            q_s, k_s, vt_s, o_s, kv_acc, z_acc, kvz_s, s_buf, m_buf, sems):
    cp_x = pltpu.make_async_copy(x_hbm, xio_s, sems.at[0])
    cp_waq = pltpu.make_async_copy(wa_qkv_hbm, wa_qkv, sems.at[1])
    cp_wao = pltpu.make_async_copy(wa_o_hbm, wa_o, sems.at[2])
    cp_wbq = pltpu.make_async_copy(wb_qkv_hbm, wb_qkv, sems.at[3])
    cp_wbo = pltpu.make_async_copy(wb_o_hbm, wb_o, sems.at[4])
    cp_x.start()
    cp_waq.start()
    cp_wao.start()
    cp_wbq.start()
    cp_wbo.start()

    def rows_of(i):
        return pl.ds(pl.multiple_of(i * TM, TM), TM)

    def a1_tile(i, x):
        rows = rows_of(i)
        xn = _layernorm(x).astype(BF16)
        q_s[rows, :] = _phi(_mm(xn, wa_qkv[:, 0:D])).astype(BF16)
        pk = _phi(_mm(xn, wa_qkv[:, D:2 * D]))
        v = _mm(xn, wa_qkv[:, 2 * D:3 * D]).astype(BF16)
        z_acc[...] += jnp.sum(pk.reshape(TM // 8, 8, D), axis=0)
        for g in range(G):
            pkt = pk[:, g * 128:(g + 1) * 128].T.astype(BF16)
            kv_acc[g] += _mm(pkt, v[:, g * 128:(g + 1) * 128])

    def a_reset():
        kv_acc[...] = jnp.zeros(kv_acc.shape, F32)
        z_acc[...] = jnp.zeros(z_acc.shape, F32)

    def a_finalize():
        r = lax.broadcasted_iota(jnp.int32, (128, 128), 0) // DH
        c = lax.broadcasted_iota(jnp.int32, (128, 128), 1) // DH
        same = r == c
        z = jnp.sum(z_acc[...], axis=0, keepdims=True)
        for g in range(G):
            zt = jnp.broadcast_to(z[:, g * 128:(g + 1) * 128], (128, 128)).T
            kvz_s[g, :, 0:128] = jnp.where(same, kv_acc[g], 0.0).astype(BF16)
            kvz_s[g, :, 128:256] = jnp.where(same, zt, 0.0).astype(BF16)

    def a2b1_tile(i, carry):
        rows = rows_of(i)
        os = []
        for g in range(G):
            nd = _mm(q_s[rows, g * 128:(g + 1) * 128], kvz_s[g])
            os.append((nd[:, 0:128] / (nd[:, 128:256] + 1e-6)).astype(BF16))
        o = jnp.concatenate(os, axis=1)
        x = x_s[rows, :] + _mm(o, wa_o[...])
        x_s[rows, :] = x
        xn = _layernorm(x).astype(BF16)
        q_s[rows, :] = (_mm(xn, wb_qkv[:, 0:D]) * QSCALE).astype(BF16)
        k = _mm(xn, wb_qkv[:, D:2 * D]).astype(BF16)
        for g in range(G):
            k_s[g, rows, :] = k[:, g * 128:(g + 1) * 128]
        v = _mm(xn, wb_qkv[:, 2 * D:3 * D])
        vt_s[:, rows] = v.T.astype(BF16)
        return carry

    lane = lax.broadcasted_iota(jnp.int32, (TQ, 128), 1)

    def attn_group(ja, jb):
        outs = []
        for u in range(HPG):
            if ja is not None:
                ga = ja // NQ
                qoff = pl.multiple_of((ja % NQ) * TQ, TQ)
                goff = pl.multiple_of(ga * 128, 128)
                q = q_s[pl.ds(qoff, TQ), pl.ds(goff, 128)].astype(F32)
                qm = jnp.where((lane >= u * DH) & (lane < (u + 1) * DH), q, 0.0).astype(BF16)
            if jb is not None:
                hoff = pl.multiple_of((jb // NQ) * 128 + u * DH, DH)
                m = m_buf[u]
            mrun = lrun = acc = None
            for c in range(NC):
                ks = slice(c * TK, (c + 1) * TK)
                if jb is not None:
                    p = jnp.exp2(s_buf[u, ks, :] - m)
                    for r in reversed(range(TK // 16)):
                        pr = p[16 * r:16 * r + 8] + p[16 * r + 8:16 * r + 16]
                        lrun = pr if lrun is None else lrun + pr
                    ot = _mm(vt_s[pl.ds(hoff, DH), ks], p.astype(BF16))
                    acc = ot if acc is None else acc + ot
                if ja is not None:
                    st = lax.dot_general(k_s[ga, ks, :], qm, NT_DIMS,
                                         preferred_element_type=F32)
                    s_buf[u, ks, :] = st
                    mc = jnp.max(st.reshape(TK // 8, 8, TQ), axis=0)
                    mrun = mc if mrun is None else jnp.maximum(mrun, mc)
            if ja is not None:
                m_buf[u] = jnp.max(mrun, axis=0, keepdims=True)
            if jb is not None:
                l = jnp.sum(lrun, axis=0, keepdims=True)
                outs.append(acc / l)
        if jb is not None:
            qoff = pl.multiple_of((jb % NQ) * TQ, TQ)
            goff = pl.multiple_of((jb // NQ) * 128, 128)
            ot = jnp.concatenate(outs, axis=0)
            o_s[pl.ds(qoff, TQ), pl.ds(goff, 128)] = ot.T.astype(BF16)

    def attention():
        n = G * NQ
        attn_group(0, None)

        def body(j, carry):
            attn_group(j + 1, j)
            return carry

        lax.fori_loop(0, n - 1, body, 0)
        attn_group(None, n - 1)

    cp_x.wait()
    cp_waq.wait()
    a_reset()

    def first_a1(i, carry):
        x = xio_s[rows_of(i), :].astype(F32)
        x_s[rows_of(i), :] = x
        a1_tile(i, x)
        return carry

    lax.fori_loop(0, NTM, first_a1, 0)
    cp_wao.wait()
    cp_wbq.wait()
    cp_wbo.wait()

    def layer_pair(l, carry):
        a_finalize()
        lax.fori_loop(0, NTM, a2b1_tile, 0)
        attention()

        @pl.when(l == 0)
        def _():
            a_reset()

            def b3a1(i, c):
                rows = rows_of(i)
                x = x_s[rows, :] + _mm(o_s[rows, :], wb_o[...])
                x_s[rows, :] = x
                a1_tile(i, x)
                return c

            lax.fori_loop(0, NTM, b3a1, 0)

        @pl.when(l == 1)
        def _():
            def b3out(i, c):
                rows = rows_of(i)
                x = x_s[rows, :] + _mm(o_s[rows, :], wb_o[...])
                xio_s[rows, :] = x.astype(BF16)
                return c

            lax.fori_loop(0, NTM, b3out, 0)

        return carry

    lax.fori_loop(0, 2, layer_pair, 0)
    cp_out = pltpu.make_async_copy(xio_s, out_hbm, sems.at[0])
    cp_out.start()
    cp_out.wait()


@jax.jit
def pallas_interleave_layers__linear_attn_block__mha_block__prompt_kernel(
    A_x: jax.Array,
    A_wqkv: jax.Array,
    A_wo: jax.Array,
    B_x: jax.Array,
    B_wqkv: jax.Array,
    B_wo: jax.Array,
):
    del B_x
    x = A_x.reshape(S, D)
    any_spec = pl.BlockSpec(memory_space=pl.ANY)
    out = pl.pallas_call(
        _kernel,
        out_shape=jax.ShapeDtypeStruct((S, D), BF16),
        in_specs=[any_spec] * 5,
        out_specs=any_spec,
        scratch_shapes=[
            pltpu.VMEM((S, D), BF16),
            pltpu.VMEM((S, D), F32),
            pltpu.VMEM((D, 3 * D), BF16),
            pltpu.VMEM((D, D), BF16),
            pltpu.VMEM((D, 3 * D), BF16),
            pltpu.VMEM((D, D), BF16),
            pltpu.VMEM((S, D), BF16),
            pltpu.VMEM((G, S, 128), BF16),
            pltpu.VMEM((D, S), BF16),
            pltpu.VMEM((S, D), BF16),
            pltpu.VMEM((G, 128, 128), F32),
            pltpu.VMEM((8, D), F32),
            pltpu.VMEM((G, 128, 256), BF16),
            pltpu.VMEM((HPG, S, TQ), F32),
            pltpu.VMEM((HPG, 1, TQ), F32),
            pltpu.SemaphoreType.DMA((5,)),
        ],
        compiler_params=pltpu.CompilerParams(vmem_limit_bytes=110 * 1024 * 1024),
    )(x, A_wqkv, A_wo, B_wqkv, B_wo)
    return out.reshape(1, S, D)
```

```python
import functools
import math

import jax
import jax.numpy as jnp
from jax import lax
import jax.experimental.pallas as pl
import jax.experimental.pallas.tpu as pltpu

S = 2048
D = 1024
H = 32
DH = D // H
G = D // 128
HPG = 128 // DH
TM = 256
NTM = S // TM
RC = 32
NRC = TM // RC
TQ = 512
TK = 128
NQ = S // TQ
NC = S // TK
NSTEP = G * NQ
UN = 2
LAG = 3
LEADS = (4,)

F32 = jnp.float32
BF16 = jnp.bfloat16
U32 = jnp.uint32
NT_DIMS = (((1,), (1,)), ((), ()))
QSCALE = (DH ** -0.5) * math.log2(math.e)


def _recip(d):
    r = pl.reciprocal(d, approx=True)
    return r * (2.0 - d * r)


def _layernorm(x, tok=None, flag=None):
    m = jnp.mean(x, axis=-1, keepdims=True)
    if tok is not None:
        m = jnp.where(flag, tok, m)
    xc = x - m
    v = jnp.mean(xc * xc, axis=-1, keepdims=True)
    return xc * lax.rsqrt(v + 1e-5)


def _phi(t):
    return jnp.where(t > 0, t + 1.0, jnp.exp(t)) + 1e-6


def _mm(a, b):
    return jnp.dot(a, b, preferred_element_type=F32)


def _gs(g):
    return slice(g * 128, (g + 1) * 128)


def _ds(start, size, mult=None):
    if isinstance(start, int):
        return pl.ds(start, size)
    return pl.ds(pl.multiple_of(start, mult or size), size)


def _pack(x):
    return pltpu.bitcast(x.astype(BF16), U32)


def _unpack(x):
    return pltpu.bitcast(x, BF16)


def _attn_order():
    n = HPG * NC
    order = []
    bi = ai = 0
    while ai < n:
        if bi < n:
            order.append(("b", bi))
            bi += 1
            if ai in LEADS and bi < n:
                order.append(("b", bi))
                bi += 1
        order.append(("a", ai))
        ai += 1
    return order


def _kernel(x_hbm, wa_qkv_hbm, wa_o_hbm, wb_qkv_hbm, wb_o_hbm, out_hbm,
            xio_s, x_s, xn_s, wa_qkv, wa_o, wb_qkv, wb_o,
            pq_s, pkt_s, qt_s, k_s, vt_s, o_s, kv_acc, z_acc, zt_s, m_s, s_buf, m_buf,
            flag_s, x_sems, w_sems):
    def rows_of(i):
        return _ds(i * TM, TM)

    def prows_of(i):
        return _ds(i * (TM // 2), TM // 2)

    def cp_x(i):
        return pltpu.make_async_copy(x_hbm.at[rows_of(i)], xio_s.at[rows_of(i)], x_sems.at[i])

    def cp_out(i):
        return pltpu.make_async_copy(xio_s.at[rows_of(i)], out_hbm.at[rows_of(i)], x_sems.at[i])

    def cp_wa(col0, ncol, sem):
        cols = pl.ds(col0, ncol)
        return pltpu.make_async_copy(wa_qkv_hbm.at[:, cols], wa_qkv.at[:, cols], w_sems.at[sem])

    cp_waq = cp_wa(0, D, 0)
    cp_wak0 = cp_wa(D, D // 2, 1)
    cp_wak1 = cp_wa(D + D // 2, D // 2, 6)
    cp_wav = cp_wa(2 * D, D, 2)
    cp_wao = pltpu.make_async_copy(wa_o_hbm, wa_o, w_sems.at[3])
    cp_wbq = pltpu.make_async_copy(wb_qkv_hbm, wb_qkv, w_sems.at[4])
    cp_wbo = pltpu.make_async_copy(wb_o_hbm, wb_o, w_sems.at[5])

    def xn_of(i):
        return _unpack(xn_s[prows_of(i), :])

    def ln_in(i):
        x = xio_s[rows_of(i), :].astype(F32)
        xn_s[prows_of(i), :] = _pack(_layernorm(x))

    def ln_after(i, x, flag, per):
        def after(n, tok):
            for r in range(n * per, min((n + 1) * per, NRC)):
                xr = x[r * RC:(r + 1) * RC]
                xn_s[_ds(i * (TM // 2) + r * (RC // 2), RC // 2), :] = _pack(
                    _layernorm(xr, tok[0:RC, 0:1], flag))
        return after

    def resid(i, o, w, src):
        rows = rows_of(i)
        x = src[rows, :].astype(F32) + _mm(o, w)
        x_s[rows, :] = x
        return x

    def a1_k_post(k, g):
        pk = _phi(k)
        z_acc[:, _gs(g)] += jnp.sum(pk.reshape(pk.shape[0] // 8, 8, 128), axis=0)
        return pk.T.astype(BF16)

    def a1_k(xn, gs=range(G), after=None):
        out = []
        for n, g in enumerate(gs):
            k = _mm(xn, wa_qkv[:, D + g * 128:D + (g + 1) * 128])
            out.append(a1_k_post(k, g))
            if after is not None:
                after(n, k)
        return out

    def a1_k_store(xn):
        for g, pkt in enumerate(a1_k(xn)):
            pkt_s[g] = _pack(pkt)

    def a1_v(xn, pkts=None, after=None):
        vbs = []
        for g in range(G):
            v = _mm(xn, wa_qkv[:, 2 * D + g * 128:2 * D + (g + 1) * 128])
            vbs.append(v.astype(BF16))
            if after is not None:
                after(g, v)
        for g in range(G):
            pkt = _unpack(pkt_s[g]) if pkts is None else pkts[g]
            kv_acc[g] += _mm(pkt, vbs[g])

    def a1_q(i, xn, gs=range(G), after=None):
        for n, g in enumerate(gs):
            q = _mm(xn, wa_qkv[:, _gs(g)])
            pq_s[prows_of(i), _gs(g)] = _pack(_phi(q))
            if after is not None:
                after(n, q)

    def a_reset():
        kv_acc[...] = jnp.zeros(kv_acc.shape, F32)
        z_acc[...] = jnp.zeros(z_acc.shape, F32)

    def a_fin_z():
        zr = lax.broadcasted_iota(jnp.int32, (16, 128), 0)
        zc = lax.broadcasted_iota(jnp.int32, (16, 128), 1) // DH
        z = jnp.sum(z_acc[...], axis=0, keepdims=True)
        for g in range(G):
            zt_s[g] = _pack(jnp.where(zr == zc, z[:, _gs(g)], 0.0))

    def a_fin_m():
        r = lax.broadcasted_iota(jnp.int32, (128, 128), 0) // DH
        c = lax.broadcasted_iota(jnp.int32, (128, 128), 1) // DH
        same = r == c
        for g in range(G):
            kvm = jnp.where(same, kv_acc[g], 0.0).astype(BF16)
            m_s[g * 64:(g + 1) * 64, :] = _pack(_mm(kvm, wa_o[_gs(g), :]))

    def a2_pqn(i, g):
        pq = _unpack(pq_s[prows_of(i), _gs(g)])
        dent = lax.dot_general(_unpack(zt_s[g]), pq, NT_DIMS, preferred_element_type=F32)
        r = _recip(dent[0:8] + 1e-6)
        rb = jnp.concatenate(
            [jnp.broadcast_to(r[u:u + 1], (DH, TM)) for u in range(HPG)], axis=0)
        return (pq.astype(F32) * rb.T).astype(BF16)

    def b1_v(i, xn, g):
        v = _mm(xn, wb_qkv[:, 2 * D + g * 128:2 * D + (g + 1) * 128])
        vt_s[g * 64:(g + 1) * 64, rows_of(i)] = _pack(v.T)

    def b1_q(i, xn, after=None):
        for g in range(G):
            q = _mm(xn, wb_qkv[:, _gs(g)])
            qt_s[g * 64:(g + 1) * 64, rows_of(i)] = _pack((q * QSCALE).T)
            if after is not None:
                after(g, q)

    def b1_k(i, xn):
        for g in range(G):
            k_s[g, prows_of(i), :] = _pack(_mm(xn, wb_qkv[:, D + g * 128:D + (g + 1) * 128]))

    def attn_group(ja, jb, toks=None, flag=None, extra=None):
        outs = []
        sa = {}
        sb = {}
        for kind, idx in _attn_order():
            u, c = divmod(idx, NC)
            ks = slice(c * TK, (c + 1) * TK)
            if kind == "b" and jb is not None:
                if c == 0:
                    sb = dict(hrows=_ds((jb // NQ) * 64 + u * (DH // 2), DH // 2),
                              m8=m_buf[u], lrun=None, acc=None)
                m8 = sb["m8"]
                if flag is not None and len(toks) >= LAG:
                    m8 = jnp.where(flag, toks[-LAG], m8)
                p = jnp.exp2(s_buf[u, ks, :].reshape(TK // 8, 8, TQ) - m8[None]).reshape(TK, TQ)
                lrun = sb["lrun"]
                for r in reversed(range(TK // 16)):
                    pr = p[16 * r:16 * r + 8] + p[16 * r + 8:16 * r + 16]
                    lrun = pr if lrun is None else lrun + pr
                sb["lrun"] = lrun
                ot = _mm(_unpack(vt_s[sb["hrows"], ks]), p.astype(BF16))
                sb["acc"] = ot if sb["acc"] is None else sb["acc"] + ot
                if c == NC - 1:
                    l = jnp.sum(lrun, axis=0, keepdims=True)
                    outs.append(sb["acc"] * (1.0 / l))
                    if u == HPG - 1:
                        ot = jnp.concatenate(outs, axis=0)
                        o_s[_ds((jb % NQ) * (TQ // 2), TQ // 2), _ds((jb // NQ) * 128, 128)] = _pack(ot.T)
            if kind == "a" and extra is not None:
                y = extra(idx)
                if toks is not None:
                    toks.append(jnp.concatenate([y[0:8]] * (TQ // 128), axis=1))
            if kind == "a" and ja is not None:
                if c == 0:
                    ga = ja // NQ
                    qh = _unpack(qt_s[_ds(ga * 64 + u * (DH // 2), DH // 2), _ds((ja % NQ) * TQ, TQ)])
                    parts = []
                    if u > 0:
                        parts.append(jnp.zeros((u * DH, TQ), BF16))
                    parts.append(qh)
                    if u < HPG - 1:
                        parts.append(jnp.zeros(((HPG - 1 - u) * DH, TQ), BF16))
                    sa = dict(qm=jnp.concatenate(parts, axis=0), g=ga, mrun=None)
                kc = _unpack(k_s[sa["g"], c * (TK // 2):(c + 1) * (TK // 2), :])
                st = _mm(kc, sa["qm"])
                s_buf[u, ks, :] = st
                if toks is not None:
                    toks.append(st[0:8])
                mc = jnp.max(st.reshape(TK // 8, 8, TQ), axis=0)
                sa["mrun"] = mc if sa["mrun"] is None else jnp.maximum(sa["mrun"], mc)
                if c == NC - 1:
                    m_buf[u] = jnp.broadcast_to(jnp.max(sa["mrun"], axis=0, keepdims=True), (8, TQ))

    n_att_iter = (NSTEP - 1) // UN

    def attn_loop():
        def body(jj, carry):
            toks = []
            for t in range(UN):
                attn_group(UN * jj + t + 1, UN * jj + t, toks, (jj < 0) if t > 0 else None)
            return carry

        lax.fori_loop(0, n_att_iter, body, 0)

    def attn_tail(extra):
        toks = []
        flag = None
        for j in range(n_att_iter * UN, NSTEP - 1):
            attn_group(j + 1, j, toks, flag)
            flag = flag_s[0] != 0
        attn_group(None, NSTEP - 1, toks, flag, extra)

    def half_mm_pieces(lhs_of, w_ref, col0, init_of, done):
        part = []

        def piece(r):
            n, kh = divmod(r, 2)
            kk = slice(kh * 512, (kh + 1) * 512)
            y = _mm(lhs_of(kk), w_ref[kk, col0 + n * 128:col0 + (n + 1) * 128])
            if kh == 0:
                init = init_of(n)
                part.append(y if init is None else init + y)
            else:
                done(n, part.pop() + y)
            return y

        return piece

    def b3_half(h, final):
        rows = pl.ds(h * 128, 128)
        prows = pl.ds(h * 64, 64)
        cols = []

        def done(n, y):
            cols.append(y)
            if n == G - 1:
                x = jnp.concatenate(cols, axis=1)
                if final:
                    xio_s[rows, :] = x.astype(BF16)
                else:
                    x_s[rows, :] = x
                    xn_s[prows, :] = _pack(_layernorm(x))

        return half_mm_pieces(lambda kk: _unpack(o_s[prows, kk]), wb_o, 0,
                              lambda n: x_s[rows, _gs(n)], done)

    def k_half(h):
        def done(n, k):
            pkt_s[n, :, h * 128:(h + 1) * 128] = _pack(a1_k_post(k, n))

        return half_mm_pieces(lambda kk: _unpack(xn_s[pl.ds(h * 64, 64), kk]), wa_qkv, D,
                              lambda n: None, done)

    def tail_pieces(final):
        halves = [b3_half(0, final), b3_half(1, final)]
        if final:
            halves += [b3_half(2, final), b3_half(3, final)]
        else:
            halves += [k_half(0), k_half(1)]
        return lambda idx: halves[idx // 16](idx % 16)

    def a1_last_and_a2_first(src):
        i = NTM - 1
        xn = xn_of(i)
        a_fin_z()
        a1_v(xn)
        pqn = []
        for g in range(G // 2):
            a1_q(i, xn, [g])
            pqn.append(a2_pqn(0, 2 * g))
            pqn.append(a2_pqn(0, 2 * g + 1))
        a_fin_m()
        x = resid(0, jnp.concatenate(pqn, axis=1), _unpack(m_s[...]), src)
        a1_q(i, xn, range(G // 2, G), ln_after(0, x, flag_s[0] != 0, 3))

    def a2b1_body(src, i, carry):
        xn = xn_of(i)
        pqn = []
        for g in range(G):
            b1_v(i, xn, g)
            pqn.append(a2_pqn(i + 1, g))
        x = resid(i + 1, jnp.concatenate(pqn, axis=1), _unpack(m_s[...]), src)
        b1_q(i, xn, ln_after(i + 1, x, i < 0, 1))
        b1_k(i, xn)
        return carry

    def b1_last_and_attn():
        i = NTM - 1
        xn = xn_of(i)
        b1_k(i, xn)
        for g in range(G):
            b1_v(i, xn, g)
        b1_q(i, xn)
        attn_group(0, None)

    def b3a1_body(i, carry):
        xn = xn_of(i)
        x = resid(i + 1, _unpack(o_s[prows_of(i + 1), :]), wb_o[...], x_s)
        a1_v(xn, None, ln_after(i + 1, x, i < 0, 2))
        a1_k_store(xn_of(i + 1))
        a1_q(i, xn)
        return carry

    def a1_first_body(i, carry):
        cp_x(i + 1).wait()
        xn = xn_of(i)
        x = xio_s[rows_of(i + 1), :].astype(F32)
        a1_v(xn, None, ln_after(i + 1, x, i < 0, 2))
        a1_k_store(xn_of(i + 1))
        a1_q(i, xn)
        return carry

    def b3out_body(j, carry):
        for t in range(2):
            i = 2 * j + t
            rows = rows_of(i)
            x = x_s[rows, :] + _mm(_unpack(o_s[prows_of(i), :]), wb_o[...])
            xio_s[rows, :] = x.astype(BF16)
            cp_out(i).start()
        return carry

    flag_s[0] = 0
    cp_x(0).start()
    cp_wak0.start()
    a_reset()
    cp_x(0).wait()
    cp_wak1.start()
    ln_in(0)
    cp_wak0.wait()
    cp_x(1).start()
    xn = xn_of(0)
    pkts = a1_k(xn, range(G // 2))
    cp_wak1.wait()
    cp_x(1).wait()
    cp_wav.start()
    x1 = xio_s[rows_of(1), :].astype(F32)
    pkts += a1_k(xn, range(G // 2, G), ln_after(1, x1, flag_s[0] != 0, 3))
    a1_k_store(xn_of(1))
    cp_wav.wait()
    cp_waq.start()
    cp_x(2).start()
    a1_v(xn, pkts)
    cp_waq.wait()
    for i in range(3, NTM):
        cp_x(i).start()
    a1_q(0, xn)
    cp_wao.start()
    cp_wbq.start()
    cp_wbo.start()
    lax.fori_loop(1, NTM - 1, a1_first_body, 0)
    cp_wao.wait()
    cp_wbq.wait()
    cp_wbo.wait()

    for l in range(2):
        src = xio_s if l == 0 else x_s
        a1_last_and_a2_first(src)
        lax.fori_loop(0, NTM - 1, functools.partial(a2b1_body, src), 0)
        b1_last_and_attn()
        attn_loop()
        if l == 0:
            a_reset()
            attn_tail(tail_pieces(False))
            lax.fori_loop(0, NTM - 1, b3a1_body, 0)
        else:
            attn_tail(tail_pieces(True))
            cp_out(0).start()
            cp_out(1).start()
            lax.fori_loop(1, NTM // 2, b3out_body, 0)
    for i in range(NTM):
        cp_out(i).wait()


@jax.jit
def pallas_interleave_layers__linear_attn_block__mha_block__prompt_kernel(
    A_x: jax.Array,
    A_wqkv: jax.Array,
    A_wo: jax.Array,
    B_x: jax.Array,
    B_wqkv: jax.Array,
    B_wo: jax.Array,
):
    del B_x
    x = A_x.reshape(S, D)
    any_spec = pl.BlockSpec(memory_space=pl.ANY)
    out = pl.pallas_call(
        _kernel,
        out_shape=jax.ShapeDtypeStruct((S, D), BF16),
        in_specs=[any_spec] * 5,
        out_specs=any_spec,
        scratch_shapes=[
            pltpu.VMEM((S, D), BF16),
            pltpu.VMEM((S, D), F32),
            pltpu.VMEM((S // 2, D), U32),
            pltpu.VMEM((D, 3 * D), BF16),
            pltpu.VMEM((D, D), BF16),
            pltpu.VMEM((D, 3 * D), BF16),
            pltpu.VMEM((D, D), BF16),
            pltpu.VMEM((S // 2, D), U32),
            pltpu.VMEM((G, 64, TM), U32),
            pltpu.VMEM((D // 2, S), U32),
            pltpu.VMEM((G, S // 2, 128), U32),
            pltpu.VMEM((D // 2, S), U32),
            pltpu.VMEM((S // 2, D), U32),
            pltpu.VMEM((G, 128, 128), F32),
            pltpu.VMEM((8, D), F32),
            pltpu.VMEM((G, 8, 128), U32),
            pltpu.VMEM((D // 2, D), U32),
            pltpu.VMEM((HPG, S, TQ), F32),
            pltpu.VMEM((HPG, 8, TQ), F32),
            pltpu.SMEM((1,), jnp.int32),
            pltpu.SemaphoreType.DMA((NTM,)),
            pltpu.SemaphoreType.DMA((7,)),
        ],
        compiler_params=pltpu.CompilerParams(vmem_limit_bytes=110 * 1024 * 1024),
    )(x, A_wqkv, A_wo, B_wqkv, B_wo)
    return out.reshape(1, S, D)
```

```python
import functools
import math

import jax
import jax.numpy as jnp
from jax import lax
import jax.experimental.pallas as pl
import jax.experimental.pallas.tpu as pltpu

S = 2048
D = 1024
H = 32
DH = D // H
G = D // 128
HPG = 128 // DH
TM = 256
NTM = S // TM
RC = 32
NRC = TM // RC
TQ = 512
TK = 128
NQ = S // TQ
NC = S // TK
NSTEP = G * NQ
UN = 1
LAG = 3
LEADS = (4,)
NOFF = 64
KB_SLOTS = 26
TIE = 3
VT0 = 2
VT1 = 120

F32 = jnp.float32
BF16 = jnp.bfloat16
U32 = jnp.uint32
NT_DIMS = (((1,), (1,)), ((), ()))
QSCALE = (DH ** -0.5) * math.log2(math.e)


def _recip(d):
    r = pl.reciprocal(d, approx=True)
    return r * (2.0 - d * r)


def _layernorm(x, tok=None, flag=None):
    m = jnp.mean(x, axis=-1, keepdims=True)
    if tok is not None:
        m = jnp.where(flag, tok, m)
    xc = x - m
    v = jnp.mean(xc * xc, axis=-1, keepdims=True)
    return xc * lax.rsqrt(v + 1e-5)


def _phi(t):
    return jnp.where(t > 0, t + 1.0, jnp.exp(t)) + 1e-6


def _mm(a, b):
    return jnp.dot(a, b, preferred_element_type=F32)


def _gs(g):
    return slice(g * 128, (g + 1) * 128)


def _ds(start, size, mult=None):
    if isinstance(start, int):
        return pl.ds(start, size)
    return pl.ds(pl.multiple_of(start, mult or size), size)


def _pack(x):
    return pltpu.bitcast(x.astype(BF16), U32)


def _unpack(x):
    return pltpu.bitcast(x, BF16)


def _a_chunks(first):
    if first:
        sizes = [TK - NOFF] + [TK] * (NC - 1)
    else:
        sizes = [TK] * NC
        n = NOFF // 16
        for i in range(n):
            sizes[(i * NC) // n] -= 16
    return [(NOFF + sum(sizes[:i]), sizes[i]) for i in range(NC)]


def _attn_order():
    n = HPG * NC
    order = []
    bi = ai = 0
    while ai < n:
        if bi < n:
            order.append(("b", bi))
            bi += 1
            if ai in LEADS and bi < n:
                order.append(("b", bi))
                bi += 1
        order.append(("a", ai))
        ai += 1
    return order


def _kernel(x_hbm, wa_qkv_hbm, wa_o_hbm, wb_qkv_hbm, wb_o_hbm, out_hbm,
            xio_s, x_s, xn_s, wa_qkv, wa_o, wb_qkv, wb_o,
            pq_s, pkt_s, qt_s, k_s, vt_s, o_s, kv_acc, z_acc, zt_s, m_s, s_buf, m_buf, qb_s, kb_s,
            flag_s, x_sems, w_sems):
    def rows_of(i):
        return _ds(i * TM, TM)

    def prows_of(i):
        return _ds(i * (TM // 2), TM // 2)

    def cp_x(i):
        return pltpu.make_async_copy(x_hbm.at[rows_of(i)], xio_s.at[rows_of(i)], x_sems.at[i])

    def cp_out(i):
        return pltpu.make_async_copy(xio_s.at[rows_of(i)], out_hbm.at[rows_of(i)], x_sems.at[i])

    def cp_wa(col0, ncol, sem):
        cols = pl.ds(col0, ncol)
        return pltpu.make_async_copy(wa_qkv_hbm.at[:, cols], wa_qkv.at[:, cols], w_sems.at[sem])

    cp_waq = cp_wa(0, D, 0)
    cp_wak0 = cp_wa(D, D // 2, 1)
    cp_wak1 = cp_wa(D + D // 2, D // 2, 6)
    cp_wav = cp_wa(2 * D, D, 2)
    cp_wao = pltpu.make_async_copy(wa_o_hbm, wa_o, w_sems.at[3])
    cp_wbq = pltpu.make_async_copy(wb_qkv_hbm, wb_qkv, w_sems.at[4])
    cp_wbo = pltpu.make_async_copy(wb_o_hbm, wb_o, w_sems.at[5])

    def xn_of(i):
        return _unpack(xn_s[prows_of(i), :])

    def ln_in(i):
        x = xio_s[rows_of(i), :].astype(F32)
        xn_s[prows_of(i), :] = _pack(_layernorm(x))

    def ln_after(i, x, flag, per):
        def after(n, tok):
            for r in range(n * per, min((n + 1) * per, NRC)):
                xr = x[r * RC:(r + 1) * RC]
                xn_s[_ds(i * (TM // 2) + r * (RC // 2), RC // 2), :] = _pack(
                    _layernorm(xr, tok[0:RC, 0:1], flag))
        return after

    def resid(i, o, w, src):
        rows = rows_of(i)
        x = src[rows, :].astype(F32) + _mm(o, w)
        x_s[rows, :] = x
        return x

    def a1_k_post(k, g):
        pk = _phi(k)
        z_acc[:, _gs(g)] += jnp.sum(pk.reshape(pk.shape[0] // 8, 8, 128), axis=0)
        return pk.T.astype(BF16)

    def a1_k(xn, gs=range(G), after=None):
        out = []
        for n, g in enumerate(gs):
            k = _mm(xn, wa_qkv[:, D + g * 128:D + (g + 1) * 128])
            out.append(a1_k_post(k, g))
            if after is not None:
                after(n, k)
        return out

    def a1_k_store(xn):
        for g, pkt in enumerate(a1_k(xn)):
            pkt_s[g] = _pack(pkt)

    def a1_v(xn, pkts=None, after=None):
        vbs = []
        for g in range(G):
            v = _mm(xn, wa_qkv[:, 2 * D + g * 128:2 * D + (g + 1) * 128])
            vbs.append(v.astype(BF16))
            if after is not None:
                after(g, v)
        for g in range(G):
            pkt = _unpack(pkt_s[g]) if pkts is None else pkts[g]
            kv_acc[g] += _mm(pkt, vbs[g])

    def a1_q(i, xn, gs=range(G), after=None):
        for n, g in enumerate(gs):
            q = _mm(xn, wa_qkv[:, _gs(g)])
            pq_s[prows_of(i), _gs(g)] = _pack(_phi(q))
            if after is not None:
                after(n, q)

    def a_reset():
        kv_acc[...] = jnp.zeros(kv_acc.shape, F32)
        z_acc[...] = jnp.zeros(z_acc.shape, F32)

    def a_fin_z():
        zr = lax.broadcasted_iota(jnp.int32, (16, 128), 0)
        zc = lax.broadcasted_iota(jnp.int32, (16, 128), 1) // DH
        z = jnp.sum(z_acc[...], axis=0, keepdims=True)
        for g in range(G):
            zt_s[g] = _pack(jnp.where(zr == zc, z[:, _gs(g)], 0.0))

    def a_fin_m():
        r = lax.broadcasted_iota(jnp.int32, (128, 128), 0) // DH
        c = lax.broadcasted_iota(jnp.int32, (128, 128), 1) // DH
        same = r == c
        for g in range(G):
            kvm = jnp.where(same, kv_acc[g], 0.0).astype(BF16)
            m_s[g * 64:(g + 1) * 64, :] = _pack(_mm(kvm, wa_o[_gs(g), :]))

    def a2_pqn(i, g):
        pq = _unpack(pq_s[prows_of(i), _gs(g)])
        dent = lax.dot_general(_unpack(zt_s[g]), pq, NT_DIMS, preferred_element_type=F32)
        r = _recip(dent[0:8] + 1e-6)
        rb = jnp.concatenate(
            [jnp.broadcast_to(r[u:u + 1], (DH, TM)) for u in range(HPG)], axis=0)
        return (pq.astype(F32) * rb.T).astype(BF16)

    def b1_v(i, xn, g):
        v = _mm(xn, wb_qkv[:, 2 * D + g * 128:2 * D + (g + 1) * 128])
        vt_s[g * 64:(g + 1) * 64, rows_of(i)] = _pack(v.T)
        return v

    def b1_q(i, xn, after=None):
        for g in range(G):
            q = _mm(xn, wb_qkv[:, _gs(g)])
            qt_s[g * 64:(g + 1) * 64, rows_of(i)] = _pack((q * QSCALE).T)
            if after is not None:
                after(g, q)

    def b1_k(i, xn, after=None):
        for g in range(G):
            k = _mm(xn, wb_qkv[:, D + g * 128:D + (g + 1) * 128])
            k_s[g, prows_of(i), :] = _pack(k)
            if after is not None:
                after(g, k)

    def kb_maker(g, flag, nslots):
        k32 = k_s[g, 0:NOFF // 2, :]
        state = {"slot": 0}

        def step(tok):
            s = state["slot"]
            state["slot"] += 1
            if NOFF == 0 or s >= nslots:
                return
            kk = jnp.where(flag, pltpu.bitcast(tok[0:NOFF // 2], U32), k32)
            kk = _unpack(kk).astype(F32)
            for d in range((s * 128) // nslots, ((s + 1) * 128) // nslots):
                kb_s[g, d] = jnp.broadcast_to(kk[:, d:d + 1], (NOFF, 128))

        return step

    def attn_group(ja, jb, toks, flag, pace_b, extra=None, prev_acc=None):
        outs = []
        sa = {}
        sb = {"acc": prev_acc}
        nunits = (NOFF // 16) * DH
        for kind, idx in _attn_order():
            u, c = divmod(idx, NC)
            ks = slice(c * TK, (c + 1) * TK)
            if kind == "b" and jb is not None:
                if c == 0:
                    prev = sb["acc"]
                    sb = dict(hrows=_ds((jb // NQ) * 64 + u * (DH // 2), DH // 2),
                              m8=m_buf[u], lrun=None,
                              acc=None if prev is None else jnp.where(flag, prev, 0.0))
                m8 = sb["m8"]
                if pace_b and len(toks) >= LAG:
                    m8 = jnp.where(flag, toks[-LAG], m8)
                p = jnp.exp2(s_buf[u, ks, :].reshape(TK // 8, 8, TQ) - m8[None]).reshape(TK, TQ)
                lrun = sb["lrun"]
                for r in reversed(range(TK // 16)):
                    pr = p[16 * r:16 * r + 8] + p[16 * r + 8:16 * r + 16]
                    lrun = pr if lrun is None else lrun + pr
                sb["lrun"] = lrun
                ot = _mm(_unpack(vt_s[sb["hrows"], ks]), p.astype(BF16))
                sb["acc"] = ot if sb["acc"] is None else sb["acc"] + ot
                if c == NC - 1:
                    l = jnp.sum(lrun, axis=0, keepdims=True)
                    outs.append(sb["acc"] * (1.0 / l))
                    if u == HPG - 1:
                        ot = jnp.concatenate(outs, axis=0)
                        o_s[_ds((jb % NQ) * (TQ // 2), TQ // 2), _ds((jb // NQ) * 128, 128)] = _pack(ot.T)
            if kind == "a" and extra is not None:
                y = extra(idx)
                toks.append(jnp.concatenate([y[0:8]] * (TQ // 128), axis=1))
            if kind == "a" and ja is not None:
                if c == 0:
                    ga = ja // NQ
                    qh = _unpack(qt_s[_ds(ga * 64 + u * (DH // 2), DH // 2), _ds((ja % NQ) * TQ, TQ)])
                    if NOFF:
                        qf = qh.astype(F32)
                        for d in range(DH):
                            qb_s[u, d] = jnp.broadcast_to(qf[d:d + 1], (8, TQ))
                    parts = []
                    if u > 0:
                        parts.append(jnp.zeros((u * DH, TQ), BF16))
                    parts.append(qh)
                    if u < HPG - 1:
                        parts.append(jnp.zeros(((HPG - 1 - u) * DH, TQ), BF16))
                    sa = dict(qm=jnp.concatenate(parts, axis=0), g=ga, mrun=None, nt=0, unit=0, sv=None)
                r0, nm = _a_chunks(u == 0)[c]
                kc = _unpack(k_s[sa["g"], r0 // 2:(r0 + nm) // 2, :])
                st = _mm(kc, sa["qm"])
                s_buf[u, r0:r0 + nm, :] = st
                toks.append(st[0:8])
                mc = jnp.max(st.reshape(nm // 8, 8, TQ), axis=0)
                for r in range(nm // 16):
                    t = sa["nt"]
                    sa["nt"] += 1
                    span = VT1 - VT0
                    upto = 0 if t < VT0 else min(nunits, ((t - VT0 + 1) * nunits + span - 1) // span)
                    while sa["unit"] < upto:
                        blk, d = divmod(sa["unit"], DH)
                        kb = kb_s[sa["g"], u * DH + d, blk * 16:(blk + 1) * 16, :]
                        k0, k1 = kb[0:8], kb[8:16]
                        tok = st[16 * r:16 * r + 8, 0:128]
                        if TIE in (1, 2) or d % 2 == 0:
                            k0 = jnp.where(flag, tok, k0)
                        if TIE == 2 or (d % 2 == 1 and TIE == 3):
                            k1 = jnp.where(flag, tok, k1)
                        qb = qb_s[u, d]
                        tt = jnp.concatenate(
                            [jnp.concatenate([k0] * (TQ // 128), axis=1) * qb,
                             jnp.concatenate([k1] * (TQ // 128), axis=1) * qb], axis=0)
                        sa["sv"] = tt if d == 0 else sa["sv"] + tt
                        if d == DH - 1:
                            sv = sa["sv"]
                            s_buf[u, blk * 16:(blk + 1) * 16, :] = sv
                            mc = jnp.maximum(mc, jnp.maximum(sv[0:8], sv[8:16]))
                        sa["unit"] += 1
                sa["mrun"] = mc if sa["mrun"] is None else jnp.maximum(sa["mrun"], mc)
                if c == NC - 1:
                    assert sa["unit"] == nunits
                    m_buf[u] = jnp.broadcast_to(jnp.max(sa["mrun"], axis=0, keepdims=True), (8, TQ))
        return sb["acc"]

    n_att_iter = (NSTEP - 1) // UN

    def attn_loop():
        def body(jj, carry):
            toks = []
            acc = None
            for t in range(UN):
                acc = attn_group(UN * jj + t + 1, UN * jj + t, toks, jj < 0, t > 0, None, acc)
            return carry

        lax.fori_loop(0, n_att_iter, body, 0)

    def attn_tail(extra):
        toks = []
        flag = flag_s[0] != 0
        acc = None
        pace = False
        for j in range(n_att_iter * UN, NSTEP - 1):
            acc = attn_group(j + 1, j, toks, flag, pace, None, acc)
            pace = True
        attn_group(None, NSTEP - 1, toks, flag, pace, extra, acc)

    def half_mm_pieces(lhs_of, w_ref, col0, init_of, done):
        part = []

        def piece(r):
            n, kh = divmod(r, 2)
            kk = slice(kh * 512, (kh + 1) * 512)
            y = _mm(lhs_of(kk), w_ref[kk, col0 + n * 128:col0 + (n + 1) * 128])
            if kh == 0:
                init = init_of(n)
                part.append(y if init is None else init + y)
            else:
                done(n, part.pop() + y)
            return y

        return piece

    def b3_half(h, final):
        rows = pl.ds(h * 128, 128)
        prows = pl.ds(h * 64, 64)
        cols = []

        def done(n, y):
            cols.append(y)
            if n == G - 1:
                x = jnp.concatenate(cols, axis=1)
                if final:
                    xio_s[rows, :] = x.astype(BF16)
                else:
                    x_s[rows, :] = x
                    xn_s[prows, :] = _pack(_layernorm(x))

        return half_mm_pieces(lambda kk: _unpack(o_s[prows, kk]), wb_o, 0,
                              lambda n: x_s[rows, _gs(n)], done)

    def k_half(h):
        def done(n, k):
            pkt_s[n, :, h * 128:(h + 1) * 128] = _pack(a1_k_post(k, n))

        return half_mm_pieces(lambda kk: _unpack(xn_s[pl.ds(h * 64, 64), kk]), wa_qkv, D,
                              lambda n: None, done)

    def tail_pieces(final):
        halves = [b3_half(0, final), b3_half(1, final)]
        if final:
            halves += [b3_half(2, final), b3_half(3, final)]
        else:
            halves += [k_half(0), k_half(1)]
        return lambda idx: halves[idx // 16](idx % 16)

    def a1_last_and_a2_first(src):
        i = NTM - 1
        xn = xn_of(i)
        a_fin_z()
        a1_v(xn)
        pqn = []
        for g in range(G // 2):
            a1_q(i, xn, [g])
            pqn.append(a2_pqn(0, 2 * g))
            pqn.append(a2_pqn(0, 2 * g + 1))
        a_fin_m()
        x = resid(0, jnp.concatenate(pqn, axis=1), _unpack(m_s[...]), src)
        a1_q(i, xn, range(G // 2, G), ln_after(0, x, flag_s[0] != 0, 3))
        b1_k(0, xn_of(0))

    def a2b1_body(src, i, carry):
        flag = i < 0
        xn = xn_of(i)
        kb_step = kb_maker(i, flag, KB_SLOTS)
        pqn = []
        for g in range(G):
            kb_step(b1_v(i, xn, g))
            pqn.append(a2_pqn(i + 1, g))
        x = resid(i + 1, jnp.concatenate(pqn, axis=1), _unpack(m_s[...]), src)
        for g in range(G):
            kb_step(x[:, _gs(g)])
        ln = ln_after(i + 1, x, flag, 2)

        def after_q(g, q):
            ln(g, q)
            if g >= G // 2:
                kb_step(q)

        b1_q(i, xn, after_q)
        b1_k(i + 1, xn_of(i + 1), lambda g, k: kb_step(k))
        return carry

    def b1_last_and_attn():
        i = NTM - 1
        flag = flag_s[0] != 0
        xn = xn_of(i)
        kb_step = kb_maker(G - 1, flag, 16)
        for g in range(G):
            kb_step(b1_v(i, xn, g))
        b1_q(i, xn, lambda g, q: kb_step(q))
        attn_group(0, None, [], flag, False)

    def b3a1_body(i, carry):
        xn = xn_of(i)
        x = resid(i + 1, _unpack(o_s[prows_of(i + 1), :]), wb_o[...], x_s)
        a1_v(xn, None, ln_after(i + 1, x, i < 0, 2))
        a1_k_store(xn_of(i + 1))
        a1_q(i, xn)
        return carry

    def a1_first_body(i, carry):
        cp_x(i + 1).wait()
        xn = xn_of(i)
        x = xio_s[rows_of(i + 1), :].astype(F32)
        a1_v(xn, None, ln_after(i + 1, x, i < 0, 2))
        a1_k_store(xn_of(i + 1))
        a1_q(i, xn)
        return carry

    def b3out_body(j, carry):
        for t in range(2):
            i = 2 * j + t
            rows = rows_of(i)
            x = x_s[rows, :] + _mm(_unpack(o_s[prows_of(i), :]), wb_o[...])
            xio_s[rows, :] = x.astype(BF16)
            cp_out(i).start()
        return carry

    flag_s[0] = 0
    cp_x(0).start()
    cp_wak0.start()
    a_reset()
    cp_x(0).wait()
    cp_wak1.start()
    ln_in(0)
    cp_wak0.wait()
    cp_x(1).start()
    xn = xn_of(0)
    pkts = a1_k(xn, range(G // 2))
    cp_wak1.wait()
    cp_x(1).wait()
    cp_wav.start()
    x1 = xio_s[rows_of(1), :].astype(F32)
    pkts += a1_k(xn, range(G // 2, G), ln_after(1, x1, flag_s[0] != 0, 3))
    a1_k_store(xn_of(1))
    cp_wav.wait()
    cp_waq.start()
    cp_x(2).start()
    a1_v(xn, pkts)
    cp_waq.wait()
    for i in range(3, NTM):
        cp_x(i).start()
    a1_q(0, xn)
    cp_wao.start()
    cp_wbq.start()
    cp_wbo.start()
    lax.fori_loop(1, NTM - 1, a1_first_body, 0)
    cp_wao.wait()
    cp_wbq.wait()
    cp_wbo.wait()

    for l in range(2):
        src = xio_s if l == 0 else x_s
        a1_last_and_a2_first(src)
        lax.fori_loop(0, NTM - 1, functools.partial(a2b1_body, src), 0)
        b1_last_and_attn()
        attn_loop()
        if l == 0:
            a_reset()
            attn_tail(tail_pieces(False))
            lax.fori_loop(0, NTM - 1, b3a1_body, 0)
        else:
            attn_tail(tail_pieces(True))
            cp_out(0).start()
            cp_out(1).start()
            lax.fori_loop(1, NTM // 2, b3out_body, 0)
    for i in range(NTM):
        cp_out(i).wait()


@jax.jit
def pallas_interleave_layers__linear_attn_block__mha_block__prompt_kernel(
    A_x: jax.Array,
    A_wqkv: jax.Array,
    A_wo: jax.Array,
    B_x: jax.Array,
    B_wqkv: jax.Array,
    B_wo: jax.Array,
):
    del B_x
    x = A_x.reshape(S, D)
    any_spec = pl.BlockSpec(memory_space=pl.ANY)
    out = pl.pallas_call(
        _kernel,
        out_shape=jax.ShapeDtypeStruct((S, D), BF16),
        in_specs=[any_spec] * 5,
        out_specs=any_spec,
        scratch_shapes=[
            pltpu.VMEM((S, D), BF16),
            pltpu.VMEM((S, D), F32),
            pltpu.VMEM((S // 2, D), U32),
            pltpu.VMEM((D, 3 * D), BF16),
            pltpu.VMEM((D, D), BF16),
            pltpu.VMEM((D, 3 * D), BF16),
            pltpu.VMEM((D, D), BF16),
            pltpu.VMEM((S // 2, D), U32),
            pltpu.VMEM((G, 64, TM), U32),
            pltpu.VMEM((D // 2, S), U32),
            pltpu.VMEM((G, S // 2, 128), U32),
            pltpu.VMEM((D // 2, S), U32),
            pltpu.VMEM((S // 2, D), U32),
            pltpu.VMEM((G, 128, 128), F32),
            pltpu.VMEM((8, D), F32),
            pltpu.VMEM((G, 8, 128), U32),
            pltpu.VMEM((D // 2, D), U32),
            pltpu.VMEM((HPG, S, TQ), F32),
            pltpu.VMEM((HPG, 8, TQ), F32),
            pltpu.VMEM((HPG, DH, 8, TQ), F32),
            pltpu.VMEM((G, 128, max(NOFF, 8), 128), F32),
            pltpu.SMEM((1,), jnp.int32),
            pltpu.SemaphoreType.DMA((NTM,)),
            pltpu.SemaphoreType.DMA((7,)),
        ],
        compiler_params=pltpu.CompilerParams(vmem_limit_bytes=127 * 1024 * 1024),
    )(x, A_wqkv, A_wo, B_wqkv, B_wo)
    return out.reshape(1, S, D)
```

```python
import functools
import math

import jax
import jax.numpy as jnp
from jax import lax
import jax.experimental.pallas as pl
import jax.experimental.pallas.tpu as pltpu

S = 2048
D = 1024
H = 32
DH = D // H
G = D // 128
HPG = 128 // DH
TM = 256
NTM = S // TM
RC = 32
NRC = TM // RC
TQ = 512
TK = 128
NQ = S // TQ
NC = S // TK
NSTEP = G * NQ
LEAD_AT = 4
NOFF = 80
VSPAN = 120
KB_SLOTS = 26
PK = 256
GAP = 2
DEN_SCHED = (2, 1, 2, 1, 1, 1, 0, 0)

F32 = jnp.float32
BF16 = jnp.bfloat16
U32 = jnp.uint32
NT_DIMS = (((1,), (1,)), ((), ()))
QSCALE = (DH ** -0.5) * math.log2(math.e)


def _recip(d):
    r = pl.reciprocal(d, approx=True)
    return r * (2.0 - d * r)


def _layernorm(x, tok=None, flag=None):
    m = jnp.mean(x, axis=-1, keepdims=True)
    if tok is not None:
        m = jnp.where(flag, tok, m)
    xc = x - m
    v = jnp.mean(xc * xc, axis=-1, keepdims=True)
    return xc * lax.rsqrt(v + 1e-5)


def _phi(t):
    return jnp.where(t > 0, t + 1.0, jnp.exp(t)) + 1e-6


def _mm(a, b):
    return jnp.dot(a, b, preferred_element_type=F32)


def _gs(g):
    return slice(g * 128, (g + 1) * 128)


def _ds(start, size, mult=None):
    if isinstance(start, int):
        return pl.ds(start, size)
    return pl.ds(pl.multiple_of(start, mult or size), size)


def _pack(x):
    return pltpu.bitcast(x.astype(BF16), U32)


def _unpack(x):
    return pltpu.bitcast(x, BF16)


def _a_chunks(first):
    if first:
        sizes = [TK - NOFF] + [TK] * (NC - 1)
    else:
        sizes = [TK] * NC
        n = NOFF // 16
        for i in range(n):
            sizes[(i * NC) // n + 2] -= 16
    return [(NOFF + sum(sizes[:i]), sizes[i]) for i in range(NC)]


def _attn_order():
    n = HPG * NC
    order = []
    bi = ai = 0
    while ai < n:
        if bi < n:
            order.append(("b", bi))
            bi += 1
            if ai == LEAD_AT:
                order.append(("b", bi))
                bi += 1
        order.append(("a", ai))
        ai += 1
    return order


def _kernel(x_hbm, wa_qkv_hbm, wa_o_hbm, wb_qkv_hbm, wb_o_hbm, out_hbm,
            xio_s, x_s, xn_s, wa_qkv, wa_o, wb_qkv, wb_o,
            pq_s, pkt_s, qt_s, k_s, vt_s, o_s, kv_acc, z_acc, zt_s, m_s, s_buf, m_buf, qb_s, kb_s, w0_s,
            flag_s, x_sems, w_sems):
    def rows_of(i):
        return _ds(i * TM, TM)

    def prows_of(i):
        return _ds(i * (TM // 2), TM // 2)

    def cp_x(i):
        return pltpu.make_async_copy(x_hbm.at[rows_of(i)], xio_s.at[rows_of(i)], x_sems.at[i])

    def cp_out(i):
        return pltpu.make_async_copy(xio_s.at[rows_of(i)], out_hbm.at[rows_of(i)], x_sems.at[i])

    def cp_wa(col0, ncol, sem):
        cols = pl.ds(col0, ncol)
        return pltpu.make_async_copy(wa_qkv_hbm.at[:, cols], wa_qkv.at[:, cols], w_sems.at[sem])

    cp_waq = cp_wa(0, D, 0)
    cp_wak0 = cp_wa(D, D // 2, 1)
    cp_wak1 = cp_wa(D + D // 2, D // 2, 6)
    cp_wav = cp_wa(2 * D, D, 2)
    cp_wao = pltpu.make_async_copy(wa_o_hbm, wa_o, w_sems.at[3])
    cp_wbq = pltpu.make_async_copy(wb_qkv_hbm, wb_qkv, w_sems.at[4])
    cp_wbo = pltpu.make_async_copy(wb_o_hbm, wb_o, w_sems.at[5])

    def xn_of(i):
        return _unpack(xn_s[prows_of(i), :])

    def ln_in(i):
        x = xio_s[rows_of(i), :].astype(F32)
        xn_s[prows_of(i), :] = _pack(_layernorm(x))

    def ln_after(i, x, flag, per):
        def after(n, tok):
            for r in range(n * per, min((n + 1) * per, NRC)):
                xr = x[r * RC:(r + 1) * RC]
                xn_s[_ds(i * (TM // 2) + r * (RC // 2), RC // 2), :] = _pack(
                    _layernorm(xr, tok[0:RC, 0:1], flag))
        return after

    def resid(i, o, w, src):
        rows = rows_of(i)
        x = src[rows, :].astype(F32) + _mm(o, w)
        x_s[rows, :] = x
        return x

    def wb_o_full():
        return jnp.concatenate([_unpack(w0_s[2]), wb_o[:, 128:D]], axis=1)

    def a1_k_post(k, g):
        pk = _phi(k)
        z_acc[:, _gs(g)] += jnp.sum(pk.reshape(pk.shape[0] // 8, 8, 128), axis=0)
        return pk.T.astype(BF16)

    def a1_k(xn, gs=range(G), after=None):
        out = []
        for n, g in enumerate(gs):
            k = _mm(xn, wa_qkv[:, D + g * 128:D + (g + 1) * 128])
            out.append(a1_k_post(k, g))
            if after is not None:
                after(n, k)
        return out

    def a1_k_store(xn):
        for g, pkt in enumerate(a1_k(xn)):
            pkt_s[g] = _pack(pkt)

    def a1_v(xn, pkts=None, after=None):
        vbs = []
        for g in range(G):
            if g == 0 and pkts is None:
                w = _unpack(w0_s[0])
            else:
                w = wa_qkv[:, 2 * D + g * 128:2 * D + (g + 1) * 128]
            v = _mm(xn, w)
            vbs.append(v.astype(BF16))
            if after is not None:
                after(g, v)
        for g in range(G):
            pkt = _unpack(pkt_s[g]) if pkts is None else pkts[g]
            kv_acc[g] += _mm(pkt, vbs[g])

    def a1_q(i, xn, gs=range(G), after=None):
        for n, g in enumerate(gs):
            q = _mm(xn, wa_qkv[:, _gs(g)])
            pq_s[prows_of(i), _gs(g)] = _pack(_phi(q))
            if after is not None:
                after(n, q)

    def a_reset():
        kv_acc[...] = jnp.zeros(kv_acc.shape, F32)
        z_acc[...] = jnp.zeros(z_acc.shape, F32)

    def a_fin_z():
        zr = lax.broadcasted_iota(jnp.int32, (16, 128), 0)
        zc = lax.broadcasted_iota(jnp.int32, (16, 128), 1) // DH
        z = jnp.sum(z_acc[...], axis=0, keepdims=True)
        for g in range(G):
            zt_s[g] = _pack(jnp.where(zr == zc, z[:, _gs(g)], 0.0))

    def a_fin_m():
        r = lax.broadcasted_iota(jnp.int32, (128, 128), 0) // DH
        c = lax.broadcasted_iota(jnp.int32, (128, 128), 1) // DH
        same = r == c
        for g in range(G):
            kvm = jnp.where(same, kv_acc[g], 0.0).astype(BF16)
            m_s[g * 64:(g + 1) * 64, :] = _pack(_mm(kvm, wa_o[_gs(g), :]))

    def a2_pqn(i, g):
        pq = _unpack(pq_s[prows_of(i), _gs(g)])
        dent = lax.dot_general(_unpack(zt_s[g]), pq, NT_DIMS, preferred_element_type=F32)
        r = _recip(dent[0:8] + 1e-6)
        rb = jnp.concatenate(
            [jnp.broadcast_to(r[u:u + 1], (DH, TM)) for u in range(HPG)], axis=0)
        return (pq.astype(F32) * rb.T).astype(BF16)

    def b1_v(i, xn, g):
        w = _unpack(w0_s[1]) if g == 0 else wb_qkv[:, 2 * D + g * 128:2 * D + (g + 1) * 128]
        v = _mm(xn, w)
        vt_s[g * 64:(g + 1) * 64, rows_of(i)] = _pack(v.T)
        return v

    def b1_q(i, xn, after=None):
        for g in range(G):
            q = _mm(xn, wb_qkv[:, _gs(g)])
            qt_s[g * 64:(g + 1) * 64, rows_of(i)] = _pack((q * QSCALE).T)
            if after is not None:
                after(g, q)

    def b1_k(i, xn, after=None):
        for g in range(G):
            k = _mm(xn, wb_qkv[:, D + g * 128:D + (g + 1) * 128])
            k_s[g, prows_of(i), :] = _pack(k)
            if after is not None:
                after(g, k)

    def kb_maker(g, flag, nslots):
        k32 = k_s[g, 0:NOFF // 2, :]
        state = {"slot": 0}

        def step(tok):
            s = state["slot"]
            state["slot"] += 1
            if s >= nslots:
                return
            kk = jnp.where(flag, pltpu.bitcast(tok[0:NOFF // 2], U32), k32)
            kk = _unpack(kk).astype(F32)
            for d in range((s * 128) // nslots, ((s + 1) * 128) // nslots):
                kb_s[g, d] = jnp.broadcast_to(kk[:, d:d + 1], (NOFF, 128))

        return step

    def attn_group(ja, jb, flag, extra=None):
        outs = []
        sa = {}
        sb = {"acc": None}
        nunits = (NOFF // 16) * DH
        for kind, idx in _attn_order():
            u, c = divmod(idx, NC)
            ks = slice(c * TK, (c + 1) * TK)
            if kind == "b" and jb is not None:
                if c == 0:
                    prev = sb["acc"]
                    sb = dict(hrows=_ds((jb // NQ) * 64 + u * (DH // 2), DH // 2),
                              m8=m_buf[u], lrun=None,
                              acc=None if prev is None else jnp.where(flag, prev, 0.0))
                p = jnp.exp2(s_buf[u, ks, :].reshape(TK // 8, 8, TQ) - sb["m8"][None]).reshape(TK, TQ)
                lrun = sb["lrun"]
                for r in reversed(range(TK // 16)):
                    pr = p[16 * r:16 * r + 8] + p[16 * r + 8:16 * r + 16]
                    lrun = pr if lrun is None else lrun + pr
                sb["lrun"] = lrun
                ot = _mm(_unpack(vt_s[sb["hrows"], ks]), p.astype(BF16))
                sb["acc"] = ot if sb["acc"] is None else sb["acc"] + ot
                if c == NC - 1:
                    l = jnp.sum(lrun, axis=0, keepdims=True)
                    outs.append(sb["acc"] * (1.0 / l))
                    if u == HPG - 1:
                        ot = jnp.concatenate(outs, axis=0)
                        o_s[_ds((jb % NQ) * (TQ // 2), TQ // 2), _ds((jb // NQ) * 128, 128)] = _pack(ot.T)
            if kind == "a" and extra is not None:
                extra(idx)
            if kind == "a" and ja is not None:
                if c == 0:
                    ga = ja // NQ
                    qh = _unpack(qt_s[_ds(ga * 64 + u * (DH // 2), DH // 2), _ds((ja % NQ) * TQ, TQ)])
                    qf = qh.astype(F32)
                    for d in range(DH):
                        qb_s[u, d] = jnp.broadcast_to(qf[d:d + 1], (8, TQ))
                    parts = []
                    if u > 0:
                        parts.append(jnp.zeros((u * DH, TQ), BF16))
                    parts.append(qh)
                    if u < HPG - 1:
                        parts.append(jnp.zeros(((HPG - 1 - u) * DH, TQ), BF16))
                    sa = dict(qm=jnp.concatenate(parts, axis=0), g=ga, mrun=None, nt=0, unit=0, sv=None)
                r0, nm = _a_chunks(u == 0)[c]
                kc = _unpack(k_s[sa["g"], r0 // 2:(r0 + nm) // 2, :])
                st = _mm(kc, sa["qm"])
                s_buf[u, r0:r0 + nm, :] = st
                mc = jnp.max(st.reshape(nm // 8, 8, TQ), axis=0)
                for r in range(nm // 16):
                    sa["nt"] += 1
                    upto = min(nunits, (sa["nt"] * nunits + VSPAN - 1) // VSPAN)
                    while sa["unit"] < upto:
                        tok = st[16 * r:16 * r + 8, 0:128]
                        blk, d = divmod(sa["unit"], DH)
                        kb = kb_s[sa["g"], u * DH + d, blk * 16:(blk + 1) * 16, :]
                        k0, k1 = kb[0:8], kb[8:16]
                        if d % 2 == 0:
                            k0 = jnp.where(flag, tok, k0)
                        else:
                            k1 = jnp.where(flag, tok, k1)
                        qb = qb_s[u, d]
                        tt = jnp.concatenate(
                            [jnp.concatenate([k0] * (TQ // 128), axis=1) * qb,
                             jnp.concatenate([k1] * (TQ // 128), axis=1) * qb], axis=0)
                        sa["sv"] = tt if d == 0 else sa["sv"] + tt
                        if d == DH - 1:
                            sv = sa["sv"]
                            s_buf[u, blk * 16:(blk + 1) * 16, :] = sv
                            mc = jnp.maximum(mc, jnp.maximum(sv[0:8], sv[8:16]))
                        sa["unit"] += 1
                sa["mrun"] = mc if sa["mrun"] is None else jnp.maximum(sa["mrun"], mc)
                if c == NC - 1:
                    assert sa["unit"] == nunits
                    m_buf[u] = jnp.broadcast_to(jnp.max(sa["mrun"], axis=0, keepdims=True), (8, TQ))

    def attn_loop():
        def body(j, carry):
            attn_group(j + 1, j, j < 0)
            return carry

        lax.fori_loop(0, NSTEP - 1, body, 0)

    def attn_tail(extra):
        attn_group(None, NSTEP - 1, flag_s[0] != 0, extra)

    def tile_mm_pieces(lhs_of, w_ref, col0, init_of, done):
        part = []
        nk = D // PK

        def piece(r):
            n, kh = divmod(r, nk)
            kk = slice(kh * PK, (kh + 1) * PK)
            y = _mm(lhs_of(kk), w_ref[kk, col0 + n * 128:col0 + (n + 1) * 128])
            if kh == 0:
                init = init_of(n)
                part.append(y if init is None else init + y)
            elif kh < nk - 1:
                part.append(part.pop() + y)
            else:
                done(n, part.pop() + y)

        return piece

    def b3_pieces(i, final):
        rows = rows_of(i)
        prows = prows_of(i)
        cols = []

        def done(n, y):
            cols.append(y)
            if n == G - 1:
                x = jnp.concatenate(cols, axis=1)
                if final:
                    xio_s[rows, :] = x.astype(BF16)
                else:
                    x_s[rows, :] = x
                    xn_s[prows, :] = _pack(_layernorm(x))

        return tile_mm_pieces(lambda kk: _unpack(o_s[prows, kk]), wb_o, 0,
                              lambda n: x_s[rows, _gs(n)], done)

    def k_pieces():
        def done(n, k):
            pkt_s[n] = _pack(a1_k_post(k, n))

        return tile_mm_pieces(lambda kk: _unpack(xn_s[prows_of(0), kk]), wa_qkv, D,
                              lambda n: None, done)

    def tail_pieces(final):
        parts = [b3_pieces(0, final), b3_pieces(1, final) if final else k_pieces()]
        gap = 0 if final else GAP

        def extra(idx):
            if idx < 32:
                todo = [idx]
            elif idx < 32 + gap:
                todo = []
            elif idx < 63:
                todo = [idx - gap]
            else:
                todo = list(range(63 - gap, 64))
            for pi in todo:
                parts[pi // 32](pi % 32)

        return extra

    def a1_last_and_a2_first(src):
        i = NTM - 1
        xn = xn_of(i)
        a_fin_z()
        a1_v(xn)
        pqn = []
        for g in range(G // 2):
            a1_q(i, xn, [g])
            pqn.append(a2_pqn(0, 2 * g))
            pqn.append(a2_pqn(0, 2 * g + 1))
        a_fin_m()
        x = resid(0, jnp.concatenate(pqn, axis=1), _unpack(m_s[...]), src)
        a1_q(i, xn, range(G // 2, G), ln_after(0, x, flag_s[0] != 0, 3))
        b1_k(0, xn_of(0))

    def a2b1_body(src, i, carry):
        flag = i < 0
        xn = xn_of(i)
        kb_step = kb_maker(i, flag, KB_SLOTS)
        pqn = []
        for g in range(G):
            kb_step(b1_v(i, xn, g))
            for _ in range(DEN_SCHED[g]):
                pqn.append(a2_pqn(i + 1, len(pqn)))
        x = resid(i + 1, jnp.concatenate(pqn, axis=1), _unpack(m_s[...]), src)
        for g in range(G):
            kb_step(x[:, _gs(g)])
        ln = ln_after(i + 1, x, flag, 2)

        def after_q(g, q):
            ln(g, q)
            if g >= G // 2:
                kb_step(q)

        b1_q(i, xn, after_q)
        b1_k(i + 1, xn_of(i + 1), lambda g, k: kb_step(k))
        return carry

    def b1_last_and_attn():
        i = NTM - 1
        flag = flag_s[0] != 0
        xn = xn_of(i)
        kb_step = kb_maker(G - 1, flag, 16)
        for g in range(G):
            kb_step(b1_v(i, xn, g))
        b1_q(i, xn, lambda g, q: kb_step(q))
        attn_group(0, None, flag)

    def b3a1_body(i, carry):
        xn = xn_of(i)
        x = resid(i + 1, _unpack(o_s[prows_of(i + 1), :]), wb_o_full(), x_s)
        a1_v(xn, None, ln_after(i + 1, x, i < 0, 2))
        a1_k_store(xn_of(i + 1))
        a1_q(i, xn)
        return carry

    def a1_first_body(i, carry):
        cp_x(i + 1).wait()
        xn = xn_of(i)
        x = xio_s[rows_of(i + 1), :].astype(F32)
        a1_v(xn, None, ln_after(i + 1, x, i < 0, 2))
        a1_k_store(xn_of(i + 1))
        a1_q(i, xn)
        return carry

    def b3out_body(j, carry):
        for t in range(2):
            i = 2 * j + t
            rows = rows_of(i)
            x = x_s[rows, :] + _mm(_unpack(o_s[prows_of(i), :]), wb_o_full())
            xio_s[rows, :] = x.astype(BF16)
            cp_out(i).start()
        return carry

    flag_s[0] = 0
    cp_x(0).start()
    cp_wak0.start()
    a_reset()
    cp_x(0).wait()
    cp_wak1.start()
    ln_in(0)
    cp_wak0.wait()
    cp_x(1).start()
    xn = xn_of(0)
    pkts = a1_k(xn, range(G // 2))
    cp_wak1.wait()
    cp_x(1).wait()
    cp_wav.start()
    x1 = xio_s[rows_of(1), :].astype(F32)
    pkts += a1_k(xn, range(G // 2, G), ln_after(1, x1, flag_s[0] != 0, 3))
    a1_k_store(xn_of(1))
    cp_wav.wait()
    cp_waq.start()
    cp_x(2).start()
    w0_s[0] = _pack(wa_qkv[:, 2 * D:2 * D + 128])
    a1_v(xn, pkts)
    cp_waq.wait()
    for i in range(3, NTM):
        cp_x(i).start()
    a1_q(0, xn)
    cp_wao.start()
    cp_wbq.start()
    cp_wbo.start()
    lax.fori_loop(1, NTM - 1, a1_first_body, 0)
    cp_wao.wait()
    cp_wbq.wait()
    cp_wbo.wait()
    w0_s[1] = _pack(wb_qkv[:, 2 * D:2 * D + 128])
    w0_s[2] = _pack(wb_o[:, 0:128])

    for l in range(2):
        src = xio_s if l == 0 else x_s
        a1_last_and_a2_first(src)
        lax.fori_loop(0, NTM - 1, functools.partial(a2b1_body, src), 0)
        b1_last_and_attn()
        attn_loop()
        if l == 0:
            a_reset()
            attn_tail(tail_pieces(False))
            lax.fori_loop(0, NTM - 1, b3a1_body, 0)
        else:
            attn_tail(tail_pieces(True))
            cp_out(0).start()
            cp_out(1).start()
            lax.fori_loop(1, NTM // 2, b3out_body, 0)
    for i in range(NTM):
        cp_out(i).wait()


@jax.jit
def pallas_interleave_layers__linear_attn_block__mha_block__prompt_kernel(
    A_x: jax.Array,
    A_wqkv: jax.Array,
    A_wo: jax.Array,
    B_x: jax.Array,
    B_wqkv: jax.Array,
    B_wo: jax.Array,
):
    del B_x
    x = A_x.reshape(S, D)
    any_spec = pl.BlockSpec(memory_space=pl.ANY)
    out = pl.pallas_call(
        _kernel,
        out_shape=jax.ShapeDtypeStruct((S, D), BF16),
        in_specs=[any_spec] * 5,
        out_specs=any_spec,
        scratch_shapes=[
            pltpu.VMEM((S, D), BF16),
            pltpu.VMEM((S, D), F32),
            pltpu.VMEM((S // 2, D), U32),
            pltpu.VMEM((D, 3 * D), BF16),
            pltpu.VMEM((D, D), BF16),
            pltpu.VMEM((D, 3 * D), BF16),
            pltpu.VMEM((D, D), BF16),
            pltpu.VMEM((S // 2, D), U32),
            pltpu.VMEM((G, 64, TM), U32),
            pltpu.VMEM((D // 2, S), U32),
            pltpu.VMEM((G, S // 2, 128), U32),
            pltpu.VMEM((D // 2, S), U32),
            pltpu.VMEM((S // 2, D), U32),
            pltpu.VMEM((G, 128, 128), F32),
            pltpu.VMEM((8, D), F32),
            pltpu.VMEM((G, 8, 128), U32),
            pltpu.VMEM((D // 2, D), U32),
            pltpu.VMEM((HPG, S, TQ), F32),
            pltpu.VMEM((HPG, 8, TQ), F32),
            pltpu.VMEM((HPG, DH, 8, TQ), F32),
            pltpu.VMEM((G, 128, NOFF, 128), F32),
            pltpu.VMEM((3, D // 2, 128), U32),
            pltpu.SMEM((1,), jnp.int32),
            pltpu.SemaphoreType.DMA((NTM,)),
            pltpu.SemaphoreType.DMA((7,)),
        ],
        compiler_params=pltpu.CompilerParams(vmem_limit_bytes=127 * 1024 * 1024),
    )(x, A_wqkv, A_wo, B_wqkv, B_wo)
    return out.reshape(1, S, D)
```

```python
import functools
import math

import jax
import jax.numpy as jnp
from jax import lax
import jax.experimental.pallas as pl
import jax.experimental.pallas.tpu as pltpu

S = 2048
D = 1024
H = 32
DH = D // H
G = D // 128
HPG = 128 // DH
TM = 256
NTM = S // TM
RC = 32
NRC = TM // RC
TQ = 512
TK = 128
NQ = S // TQ
NC = S // TK
QPS = 2
NV = QPS * HPG
SPG = NQ // QPS
NSTEP = G * SPG
LEAD_AT = 4
NOFF = 64
VSPAN = 120
KB_SLOTS = 26
PK = 256
DEN_SCHED = (2, 1, 2, 1, 1, 1, 0, 0)

F32 = jnp.float32
BF16 = jnp.bfloat16
U32 = jnp.uint32
NT_DIMS = (((1,), (1,)), ((), ()))
QSCALE = (DH ** -0.5) * math.log2(math.e)


def _recip(d):
    r = pl.reciprocal(d, approx=True)
    return r * (2.0 - d * r)


def _layernorm(x, tok=None, flag=None):
    m = jnp.mean(x, axis=-1, keepdims=True)
    if tok is not None:
        m = jnp.where(flag, tok, m)
    xc = x - m
    v = jnp.mean(xc * xc, axis=-1, keepdims=True)
    return xc * lax.rsqrt(v + 1e-5)


def _phi(t):
    return jnp.where(t > 0, t + 1.0, jnp.exp(t)) + 1e-6


def _mm(a, b):
    return jnp.dot(a, b, preferred_element_type=F32)


def _gs(g):
    return slice(g * 128, (g + 1) * 128)


def _ds(start, size, mult=None):
    if isinstance(start, int):
        return pl.ds(start, size)
    return pl.ds(pl.multiple_of(start, mult or size), size)


def _pack(x):
    return pltpu.bitcast(x.astype(BF16), U32)


def _unpack(x):
    return pltpu.bitcast(x, BF16)


def _a_chunks(first):
    if first:
        sizes = [TK - NOFF] + [TK] * (NC - 1)
    else:
        sizes = [TK] * NC
        n = NOFF // 16
        for i in range(n):
            sizes[(i * NC) // n + 1] -= 16
    return [(NOFF + sum(sizes[:i]), sizes[i]) for i in range(NC)]


def _attn_order():
    n = NV * NC
    order = []
    bi = ai = 0
    while ai < n:
        if bi < n:
            order.append(("b", bi))
            bi += 1
            if ai == LEAD_AT:
                order.append(("b", bi))
                bi += 1
        order.append(("a", ai))
        ai += 1
    return order


def _kernel(x_hbm, wa_qkv_hbm, wa_o_hbm, wb_qkv_hbm, wb_o_hbm, out_hbm,
            xio_s, x_s, xn_s, wa_qkv, wa_o, wb_qkv, wb_o,
            pq_s, pkt_s, qt_s, k_s, vt_s, kv_acc, z_acc, zt_s, m_s, s_buf, m_buf, qb_s, kb_s, w0_s,
            flag_s, x_sems, w_sems):
    o_s = pq_s

    def rows_of(i):
        return _ds(i * TM, TM)

    def prows_of(i):
        return _ds(i * (TM // 2), TM // 2)

    def cp_x(i):
        return pltpu.make_async_copy(x_hbm.at[rows_of(i)], xio_s.at[rows_of(i)], x_sems.at[i])

    def cp_out(i):
        return pltpu.make_async_copy(xio_s.at[rows_of(i)], out_hbm.at[rows_of(i)], x_sems.at[i])

    def cp_wa(col0, ncol, sem):
        cols = pl.ds(col0, ncol)
        return pltpu.make_async_copy(wa_qkv_hbm.at[:, cols], wa_qkv.at[:, cols], w_sems.at[sem])

    cp_waq = cp_wa(0, D, 0)
    cp_wak0 = cp_wa(D, D // 2, 1)
    cp_wak1 = cp_wa(D + D // 2, D // 2, 6)
    cp_wav = cp_wa(2 * D, D, 2)
    cp_wao = pltpu.make_async_copy(wa_o_hbm, wa_o, w_sems.at[3])
    cp_wbq = pltpu.make_async_copy(wb_qkv_hbm, wb_qkv, w_sems.at[4])
    cp_wbo = pltpu.make_async_copy(wb_o_hbm, wb_o, w_sems.at[5])

    def xn_of(i):
        return _unpack(xn_s[prows_of(i), :])

    def ln_in(i):
        x = xio_s[rows_of(i), :].astype(F32)
        xn_s[prows_of(i), :] = _pack(_layernorm(x))

    def ln_after(i, x, flag, per):
        def after(n, tok):
            for r in range(n * per, min((n + 1) * per, NRC)):
                xr = x[r * RC:(r + 1) * RC]
                xn_s[_ds(i * (TM // 2) + r * (RC // 2), RC // 2), :] = _pack(
                    _layernorm(xr, tok[0:RC, 0:1], flag))
        return after

    def resid(i, o, w, src):
        rows = rows_of(i)
        x = src[rows, :].astype(F32) + _mm(o, w)
        x_s[rows, :] = x
        return x

    def wb_o_full():
        return jnp.concatenate([_unpack(w0_s[2]), wb_o[:, 128:D]], axis=1)

    def a1_k_post(k, g):
        pk = _phi(k)
        z_acc[:, _gs(g)] += jnp.sum(pk.reshape(pk.shape[0] // 8, 8, 128), axis=0)
        return pk.T.astype(BF16)

    def a1_k(xn, gs=range(G), after=None):
        out = []
        for n, g in enumerate(gs):
            k = _mm(xn, wa_qkv[:, D + g * 128:D + (g + 1) * 128])
            out.append(a1_k_post(k, g))
            if after is not None:
                after(n, k)
        return out

    def a1_k_store(xn):
        for g, pkt in enumerate(a1_k(xn)):
            pkt_s[g] = _pack(pkt)

    def a1_v(xn, pkts=None, after=None):
        vbs = []
        for g in range(G):
            if g == 0 and pkts is None:
                w = _unpack(w0_s[0])
            else:
                w = wa_qkv[:, 2 * D + g * 128:2 * D + (g + 1) * 128]
            v = _mm(xn, w)
            vbs.append(v.astype(BF16))
            if after is not None:
                after(g, v)
        for g in range(G):
            pkt = _unpack(pkt_s[g]) if pkts is None else pkts[g]
            kv_acc[g] += _mm(pkt, vbs[g])

    def a1_q(i, xn, gs=range(G), after=None):
        for n, g in enumerate(gs):
            q = _mm(xn, wa_qkv[:, _gs(g)])
            pq_s[prows_of(i), _gs(g)] = _pack(_phi(q))
            if after is not None:
                after(n, q)

    def a_reset():
        kv_acc[...] = jnp.zeros(kv_acc.shape, F32)
        z_acc[...] = jnp.zeros(z_acc.shape, F32)

    def a_fin_z():
        zr = lax.broadcasted_iota(jnp.int32, (16, 128), 0)
        zc = lax.broadcasted_iota(jnp.int32, (16, 128), 1) // DH
        z = jnp.sum(z_acc[...], axis=0, keepdims=True)
        for g in range(G):
            zt_s[g] = _pack(jnp.where(zr == zc, z[:, _gs(g)], 0.0))

    def a_fin_m():
        r = lax.broadcasted_iota(jnp.int32, (128, 128), 0) // DH
        c = lax.broadcasted_iota(jnp.int32, (128, 128), 1) // DH
        same = r == c
        for g in range(G):
            kvm = jnp.where(same, kv_acc[g], 0.0).astype(BF16)
            m_s[g * 64:(g + 1) * 64, :] = _pack(_mm(kvm, wa_o[_gs(g), :]))

    def a2_pqn(i, g):
        pq = _unpack(pq_s[prows_of(i), _gs(g)])
        dent = lax.dot_general(_unpack(zt_s[g]), pq, NT_DIMS, preferred_element_type=F32)
        r = _recip(dent[0:8] + 1e-6)
        rb = jnp.concatenate(
            [jnp.broadcast_to(r[u:u + 1], (DH, TM)) for u in range(HPG)], axis=0)
        return (pq.astype(F32) * rb.T).astype(BF16)

    def b1_v(i, xn, g):
        w = _unpack(w0_s[1]) if g == 0 else wb_qkv[:, 2 * D + g * 128:2 * D + (g + 1) * 128]
        v = _mm(xn, w)
        vt_s[g * 64:(g + 1) * 64, rows_of(i)] = _pack(v.T)
        return v

    def b1_q(i, xn, after=None):
        for g in range(G):
            q = _mm(xn, wb_qkv[:, _gs(g)])
            qt_s[g * 64:(g + 1) * 64, rows_of(i)] = _pack((q * QSCALE).T)
            if after is not None:
                after(g, q)

    def b1_k(i, xn, after=None):
        for g in range(G):
            k = _mm(xn, wb_qkv[:, D + g * 128:D + (g + 1) * 128])
            k_s[g, prows_of(i), :] = _pack(k)
            if after is not None:
                after(g, k)

    def kb_maker(g, flag, nslots):
        k32 = k_s[g, 0:NOFF // 2, :]
        state = {"slot": 0}

        def step(tok):
            s = state["slot"]
            state["slot"] += 1
            if s >= nslots:
                return
            kk = jnp.where(flag, pltpu.bitcast(tok[0:NOFF // 2], U32), k32)
            kk = _unpack(kk).astype(F32)
            for d in range((s * 128) // nslots, ((s + 1) * 128) // nslots):
                kb_s[g, d] = jnp.broadcast_to(kk[:, d:d + 1], (NOFF, 128))

        return step

    def attn_group(ja, jb, flag, extra=None):
        outs = []
        sa = {}
        sb = {"acc": None}
        nunits = (NOFF // 16) * DH
        for kind, idx in _attn_order():
            v, c = divmod(idx, NC)
            t, u = divmod(v, HPG)
            ks = slice(c * TK, (c + 1) * TK)
            if kind == "b" and jb is not None:
                if c == 0:
                    prev = sb["acc"]
                    sb = dict(hrows=_ds((jb // SPG) * 64 + u * (DH // 2), DH // 2),
                              m8=m_buf[v], lrun=None,
                              acc=None if prev is None else jnp.where(flag, prev, 0.0))
                p = jnp.exp2(s_buf[v, ks, :].reshape(TK // 8, 8, TQ) - sb["m8"][None]).reshape(TK, TQ)
                lrun = sb["lrun"]
                for r in reversed(range(TK // 16)):
                    pr = p[16 * r:16 * r + 8] + p[16 * r + 8:16 * r + 16]
                    lrun = pr if lrun is None else lrun + pr
                sb["lrun"] = lrun
                ot = _mm(_unpack(vt_s[sb["hrows"], ks]), p.astype(BF16))
                sb["acc"] = ot if sb["acc"] is None else sb["acc"] + ot
                if c == NC - 1:
                    l = jnp.sum(lrun, axis=0, keepdims=True)
                    outs.append(sb["acc"] * (1.0 / l))
                    if u == HPG - 1:
                        ot = jnp.concatenate(outs, axis=0)
                        outs = []
                        qt = (jb % SPG) * QPS + t
                        o_s[_ds(qt * (TQ // 2), TQ // 2), _ds((jb // SPG) * 128, 128)] = _pack(ot.T)
            if kind == "a" and extra is not None:
                extra(idx)
            if kind == "a" and ja is not None:
                if c == 0:
                    ga = ja // SPG
                    qt = (ja % SPG) * QPS + t
                    qh = _unpack(qt_s[_ds(ga * 64 + u * (DH // 2), DH // 2), _ds(qt * TQ, TQ)])
                    qf = qh.astype(F32)
                    for d in range(DH):
                        qb_s[u, d] = jnp.broadcast_to(qf[d:d + 1], (8, TQ))
                    parts = []
                    if u > 0:
                        parts.append(jnp.zeros((u * DH, TQ), BF16))
                    parts.append(qh)
                    if u < HPG - 1:
                        parts.append(jnp.zeros(((HPG - 1 - u) * DH, TQ), BF16))
                    sa = dict(qm=jnp.concatenate(parts, axis=0), g=ga, mrun=None, nt=0, unit=0, sv=None)
                r0, nm = _a_chunks(v == 0)[c]
                kc = _unpack(k_s[sa["g"], r0 // 2:(r0 + nm) // 2, :])
                st = _mm(kc, sa["qm"])
                s_buf[v, r0:r0 + nm, :] = st
                mc = jnp.max(st.reshape(nm // 8, 8, TQ), axis=0)
                for r in range(nm // 16):
                    sa["nt"] += 1
                    upto = min(nunits, (sa["nt"] * nunits + VSPAN - 1) // VSPAN)
                    while sa["unit"] < upto:
                        tok = st[16 * r:16 * r + 8, 0:128]
                        blk, d = divmod(sa["unit"], DH)
                        kb = kb_s[sa["g"], u * DH + d, blk * 16:(blk + 1) * 16, :]
                        k0, k1 = kb[0:8], kb[8:16]
                        if d % 2 == 0:
                            k0 = jnp.where(flag, tok, k0)
                        else:
                            k1 = jnp.where(flag, tok, k1)
                        qb = qb_s[u, d]
                        tt = jnp.concatenate(
                            [jnp.concatenate([k0] * (TQ // 128), axis=1) * qb,
                             jnp.concatenate([k1] * (TQ // 128), axis=1) * qb], axis=0)
                        sa["sv"] = tt if d == 0 else sa["sv"] + tt
                        if d == DH - 1:
                            sv = sa["sv"]
                            s_buf[v, blk * 16:(blk + 1) * 16, :] = sv
                            mc = jnp.maximum(mc, jnp.maximum(sv[0:8], sv[8:16]))
                        sa["unit"] += 1
                sa["mrun"] = mc if sa["mrun"] is None else jnp.maximum(sa["mrun"], mc)
                if c == NC - 1:
                    assert sa["unit"] == nunits
                    m_buf[v] = jnp.broadcast_to(jnp.max(sa["mrun"], axis=0, keepdims=True), (8, TQ))

    def attn_loop():
        def body(j, carry):
            attn_group(j + 1, j, j < 0)
            return carry

        lax.fori_loop(0, NSTEP - 1, body, 0)

    def tile_mm_pieces(lhs_of, w_ref, col0, init_of, done):
        part = []
        nk = D // PK

        def piece(r):
            n, kh = divmod(r, nk)
            kk = slice(kh * PK, (kh + 1) * PK)
            y = _mm(lhs_of(kk), w_ref[kk, col0 + n * 128:col0 + (n + 1) * 128])
            if kh == 0:
                part.append(init_of(n) + y)
            elif kh < nk - 1:
                part.append(part.pop() + y)
            else:
                done(n, part.pop() + y)

        return piece

    def b3_pieces(i, finish, after=None):
        cols = []

        def done(n, y):
            cols.append(y)
            if after is not None:
                after(n, y)
            if n == G - 1:
                finish(jnp.concatenate(cols, axis=1))

        return tile_mm_pieces(lambda kk: _unpack(o_s[prows_of(i), kk]), wb_o, 0,
                              lambda n: x_s[rows_of(i), _gs(n)], done)

    def attn_tail_final():
        def finish(i):
            def f(x):
                xio_s[rows_of(i), :] = x.astype(BF16)
            return f

        parts = [b3_pieces(i, finish(i)) for i in range(2 * QPS)]
        attn_group(None, NSTEP - 1, flag_s[0] != 0, lambda idx: parts[idx // 32](idx % 32))

    def attn_tail_mid():
        flag = flag_s[0] != 0
        lns = {}
        pkts = []
        vbs = []

        def finish(i):
            def f(x):
                x_s[rows_of(i), :] = x
                lns[i] = ln_after(i, x, flag, 2)
            return f

        def k_done(n, k):
            lns[1](n, k)
            pkts.append(a1_k_post(k, n))

        def xn0(kk):
            return _unpack(xn_s[prows_of(0), kk])

        def zero(n):
            return jnp.where(flag, x_s[rows_of(2), _gs(n)], 0.0)

        parts = [
            b3_pieces(0, finish(0)),
            b3_pieces(1, finish(1), lambda n, y: lns[0](n, y)),
            tile_mm_pieces(xn0, wa_qkv, D, zero, k_done),
            tile_mm_pieces(xn0, wa_qkv, 2 * D, zero, lambda n, v: vbs.append(v.astype(BF16))),
        ]
        attn_group(None, NSTEP - 1, flag, lambda idx: parts[idx // 32](idx % 32))
        a1_k_store(xn_of(1))
        for g in range(G):
            kv_acc[g] += _mm(pkts[g], vbs[g])
        a1_q(0, xn_of(0))

    def a1_last_and_a2_first(src):
        i = NTM - 1
        xn = xn_of(i)
        a_fin_z()
        a1_v(xn)
        pqn = []
        for g in range(G // 2):
            a1_q(i, xn, [g])
            pqn.append(a2_pqn(0, 2 * g))
            pqn.append(a2_pqn(0, 2 * g + 1))
        a_fin_m()
        x = resid(0, jnp.concatenate(pqn, axis=1), _unpack(m_s[...]), src)
        a1_q(i, xn, range(G // 2, G), ln_after(0, x, flag_s[0] != 0, 3))
        b1_k(0, xn_of(0))

    def a2b1_body(src, i, carry):
        flag = i < 0
        xn = xn_of(i)
        kb_step = kb_maker(i, flag, KB_SLOTS)
        pqn = []
        for g in range(G):
            kb_step(b1_v(i, xn, g))
            for _ in range(DEN_SCHED[g]):
                pqn.append(a2_pqn(i + 1, len(pqn)))
        x = resid(i + 1, jnp.concatenate(pqn, axis=1), _unpack(m_s[...]), src)
        for g in range(G):
            kb_step(x[:, _gs(g)])
        ln = ln_after(i + 1, x, flag, 2)

        def after_q(g, q):
            ln(g, q)
            if g >= G // 2:
                kb_step(q)

        b1_q(i, xn, after_q)
        b1_k(i + 1, xn_of(i + 1), lambda g, k: kb_step(k))
        return carry

    def b1_last_and_attn():
        i = NTM - 1
        flag = flag_s[0] != 0
        xn = xn_of(i)
        kb_step = kb_maker(G - 1, flag, 16)
        for g in range(G):
            kb_step(b1_v(i, xn, g))
        b1_q(i, xn, lambda g, q: kb_step(q))
        attn_group(0, None, flag)

    def b3a1_body(i, carry):
        xn = xn_of(i)
        x = resid(i + 1, _unpack(o_s[prows_of(i + 1), :]), wb_o_full(), x_s)
        a1_v(xn, None, ln_after(i + 1, x, i < 0, 2))
        a1_k_store(xn_of(i + 1))
        a1_q(i, xn)
        return carry

    def a1_first_body(i, carry):
        cp_x(i + 1).wait()
        xn = xn_of(i)
        x = xio_s[rows_of(i + 1), :].astype(F32)
        a1_v(xn, None, ln_after(i + 1, x, i < 0, 2))
        a1_k_store(xn_of(i + 1))
        a1_q(i, xn)
        return carry

    def b3out_body(j, carry):
        for t in range(2):
            i = 2 * j + t
            rows = rows_of(i)
            x = x_s[rows, :] + _mm(_unpack(o_s[prows_of(i), :]), wb_o_full())
            xio_s[rows, :] = x.astype(BF16)
            cp_out(i).start()
        return carry

    flag_s[0] = 0
    flag = flag_s[0] != 0

    def k_raw(xn, g):
        return _mm(xn, wa_qkv[:, D + g * 128:D + (g + 1) * 128])

    cp_x(0).start()
    cp_wak0.start()
    a_reset()
    cp_x(0).wait()
    cp_x(1).start()
    ln_in(0)
    cp_wak0.wait()
    cp_wak1.start()
    xn = xn_of(0)
    pkts = a1_k(xn, [0])
    k = k_raw(xn, 1)
    cp_x(1).wait()
    pkts.append(a1_k_post(k, 1))
    x1 = xio_s[rows_of(1), :].astype(F32)
    xn_s[prows_of(1), :] = _pack(_layernorm(x1))
    pkts += a1_k(xn, [2, 3])
    xn1 = xn_of(1)
    for g in range(3):
        pkt_s[g] = _pack(a1_k(xn1, [g])[0])
        if g == 0:
            cp_wav.start()
    k = k_raw(xn1, 3)
    cp_wak1.wait()
    pkt_s[3] = _pack(a1_k_post(k, 3))
    pkts += a1_k(xn, range(G // 2, G))
    for g in range(G // 2, G - 1):
        pkt_s[g] = _pack(a1_k(xn1, [g])[0])
        if g == G // 2:
            cp_waq.start()
    k = k_raw(xn1, G - 1)
    cp_wav.wait()
    cp_x(2).start()
    pkt_s[G - 1] = _pack(a1_k_post(k, G - 1))
    w0_s[0] = _pack(wa_qkv[:, 2 * D:2 * D + 128])
    vbs = [_mm(xn, wa_qkv[:, 2 * D + g * 128:2 * D + (g + 1) * 128]).astype(BF16) for g in range(G)]
    cp_waq.wait()
    for i in range(3, NTM):
        cp_x(i).start()
    a1_q(0, xn, range(2))
    for g in range(G):
        kv_acc[g] += _mm(pkts[g], vbs[g])
    a1_q(0, xn, range(2, G))
    cp_wao.start()
    cp_wbq.start()
    cp_wbo.start()
    lax.fori_loop(1, NTM - 1, a1_first_body, 0)
    cp_wao.wait()
    cp_wbq.wait()
    cp_wbo.wait()
    w0_s[1] = _pack(wb_qkv[:, 2 * D:2 * D + 128])
    w0_s[2] = _pack(wb_o[:, 0:128])

    for l in range(2):
        src = xio_s if l == 0 else x_s
        a1_last_and_a2_first(src)
        lax.fori_loop(0, NTM - 1, functools.partial(a2b1_body, src), 0)
        b1_last_and_attn()
        attn_loop()
        if l == 0:
            a_reset()
            attn_tail_mid()
            lax.fori_loop(1, NTM - 1, b3a1_body, 0)
        else:
            attn_tail_final()
            for i in range(2 * QPS):
                cp_out(i).start()
            lax.fori_loop(QPS, NTM // 2, b3out_body, 0)
    for i in range(NTM):
        cp_out(i).wait()


@jax.jit
def pallas_interleave_layers__linear_attn_block__mha_block__prompt_kernel(
    A_x: jax.Array,
    A_wqkv: jax.Array,
    A_wo: jax.Array,
    B_x: jax.Array,
    B_wqkv: jax.Array,
    B_wo: jax.Array,
):
    del B_x
    x = A_x.reshape(S, D)
    any_spec = pl.BlockSpec(memory_space=pl.ANY)
    out = pl.pallas_call(
        _kernel,
        out_shape=jax.ShapeDtypeStruct((S, D), BF16),
        in_specs=[any_spec] * 5,
        out_specs=any_spec,
        scratch_shapes=[
            pltpu.VMEM((S, D), BF16),
            pltpu.VMEM((S, D), F32),
            pltpu.VMEM((S // 2, D), U32),
            pltpu.VMEM((D, 3 * D), BF16),
            pltpu.VMEM((D, D), BF16),
            pltpu.VMEM((D, 3 * D), BF16),
            pltpu.VMEM((D, D), BF16),
            pltpu.VMEM((S // 2, D), U32),
            pltpu.VMEM((G, 64, TM), U32),
            pltpu.VMEM((D // 2, S), U32),
            pltpu.VMEM((G, S // 2, 128), U32),
            pltpu.VMEM((D // 2, S), U32),
            pltpu.VMEM((G, 128, 128), F32),
            pltpu.VMEM((8, D), F32),
            pltpu.VMEM((G, 8, 128), U32),
            pltpu.VMEM((D // 2, D), U32),
            pltpu.VMEM((NV, S, TQ), F32),
            pltpu.VMEM((NV, 8, TQ), F32),
            pltpu.VMEM((HPG, DH, 8, TQ), F32),
            pltpu.VMEM((G, 128, NOFF, 128), F32),
            pltpu.VMEM((3, D // 2, 128), U32),
            pltpu.SMEM((1,), jnp.int32),
            pltpu.SemaphoreType.DMA((NTM,)),
            pltpu.SemaphoreType.DMA((7,)),
        ],
        compiler_params=pltpu.CompilerParams(vmem_limit_bytes=128 * 1024 * 1024),
    )(x, A_wqkv, A_wo, B_wqkv, B_wo)
    return out.reshape(1, S, D)
```

```python
import functools
import math

import jax
import jax.numpy as jnp
from jax import lax
import jax.experimental.pallas as pl
import jax.experimental.pallas.tpu as pltpu

S = 2048
D = 1024
H = 32
DH = D // H
G = D // 128
HPG = 128 // DH
TM = 256
NTM = S // TM
RC = 32
NRC = TM // RC
TQ = 512
TK = 128
NQ = S // TQ
NC = S // TK
QPS = 2
NV = QPS * HPG
SPG = NQ // QPS
NSTEP = G * SPG
LEAD_AT = 4
NOFF = 64
VSPAN = 120
KB_SLOTS = 26
PK = 256
DEN_SCHED = (2, 1, 2, 1, 1, 1, 0, 0)

F32 = jnp.float32
BF16 = jnp.bfloat16
U32 = jnp.uint32
NT_DIMS = (((1,), (1,)), ((), ()))
QSCALE = (DH ** -0.5) * math.log2(math.e)


def _recip(d):
    r = pl.reciprocal(d, approx=True)
    return r * (2.0 - d * r)


def _layernorm(x, tok=None, flag=None):
    m = jnp.mean(x, axis=-1, keepdims=True)
    if tok is not None:
        m = jnp.where(flag, tok, m)
    xc = x - m
    v = jnp.mean(xc * xc, axis=-1, keepdims=True)
    return xc * lax.rsqrt(v + 1e-5)


def _phi(t):
    return jnp.where(t > 0, t + 1.0, jnp.exp(t)) + 1e-6


def _mm(a, b):
    return jnp.dot(a, b, preferred_element_type=F32)


def _gs(g):
    return slice(g * 128, (g + 1) * 128)


def _ds(start, size, mult=None):
    if isinstance(start, int):
        return pl.ds(start, size)
    return pl.ds(pl.multiple_of(start, mult or size), size)


def _pack(x):
    return pltpu.bitcast(x.astype(BF16), U32)


def _unpack(x):
    return pltpu.bitcast(x, BF16)


def _a_chunks(first):
    if first:
        sizes = [TK - NOFF] + [TK] * (NC - 1)
    else:
        sizes = [TK] * NC
        n = NOFF // 16
        for i in range(n):
            sizes[(i * NC) // n + 1] -= 16
    return [(NOFF + sum(sizes[:i]), sizes[i]) for i in range(NC)]


def _attn_order():
    n = NV * NC
    order = []
    bi = ai = 0
    while ai < n:
        if bi < n:
            order.append(("b", bi))
            bi += 1
            if ai == LEAD_AT:
                order.append(("b", bi))
                bi += 1
        order.append(("a", ai))
        ai += 1
    return order


def _kernel(x_hbm, wa_qkv_hbm, wa_o_hbm, wb_qkv_hbm, wb_o_hbm, out_hbm,
            xio_s, x_s, xn_s, wa_qkv, wa_o, wb_qkv, wb_o,
            pq_s, pkt_s, qt_s, k_s, vt_s, kv_acc, z_acc, zt_s, m_s, s_buf, m_buf, qb_s, kb_s, w0_s,
            flag_s, x_sems, w_sems):
    o_s = pq_s

    def rows_of(i):
        return _ds(i * TM, TM)

    def prows_of(i):
        return _ds(i * (TM // 2), TM // 2)

    def cp_x(i):
        return pltpu.make_async_copy(x_hbm.at[rows_of(i)], xio_s.at[rows_of(i)], x_sems.at[i])

    def cp_out(i):
        return pltpu.make_async_copy(xio_s.at[rows_of(i)], out_hbm.at[rows_of(i)], x_sems.at[i])

    def cp_last(h):
        rows = pl.ds(S - TM + h * (TM // 2), TM // 2)
        return pltpu.make_async_copy(xio_s.at[rows], out_hbm.at[rows], x_sems.at[NTM - 1 + h])

    def cp_wa(col0, ncol, sem):
        cols = pl.ds(col0, ncol)
        return pltpu.make_async_copy(wa_qkv_hbm.at[:, cols], wa_qkv.at[:, cols], w_sems.at[sem])

    cp_waq = cp_wa(0, D, 0)
    cp_wak0 = cp_wa(D, D // 2, 1)
    cp_wak1 = cp_wa(D + D // 2, D // 2, 6)
    cp_wav = cp_wa(2 * D, D, 2)
    cp_wao = pltpu.make_async_copy(wa_o_hbm, wa_o, w_sems.at[3])
    cp_wbq = pltpu.make_async_copy(wb_qkv_hbm, wb_qkv, w_sems.at[4])
    cp_wbo = pltpu.make_async_copy(wb_o_hbm, wb_o, w_sems.at[5])

    def xn_of(i):
        del i
        return _unpack(xn_s[...])

    def ln_in(i):
        x = xio_s[rows_of(i), :].astype(F32)
        xn_s[...] = _pack(_layernorm(x))

    def ln_after(i, x, flag, per):
        def after(n, tok):
            for r in range(n * per, min((n + 1) * per, NRC)):
                xr = x[r * RC:(r + 1) * RC]
                xn_s[pl.ds(r * (RC // 2), RC // 2), :] = _pack(
                    _layernorm(xr, tok[0:RC, 0:1], flag))
        return after

    def resid(i, o, w, src):
        rows = rows_of(i)
        x = src[rows, :].astype(F32) + _mm(o, w)
        x_s[rows, :] = x
        return x

    def wb_o_full():
        return jnp.concatenate([_unpack(w0_s[2]), wb_o[:, 128:D]], axis=1)

    def a1_k_post(k, g):
        pk = _phi(k)
        z_acc[:, _gs(g)] += jnp.sum(pk.reshape(pk.shape[0] // 8, 8, 128), axis=0)
        return pk.T.astype(BF16)

    def k_raw(xn, g):
        return _mm(xn, wa_qkv[:, D + g * 128:D + (g + 1) * 128])

    def a1_k(xn, gs=range(G)):
        return [a1_k_post(k_raw(xn, g), g) for g in gs]

    def a1_k_store(xn):
        for g, pkt in enumerate(a1_k(xn)):
            pkt_s[g] = _pack(pkt)

    def a1_v(xn, after=None):
        vbs = []
        for g in range(G):
            w = _unpack(w0_s[0]) if g == 0 else wa_qkv[:, 2 * D + g * 128:2 * D + (g + 1) * 128]
            v = _mm(xn, w)
            vbs.append(v.astype(BF16))
            if after is not None:
                after(g, v)
        for g in range(G):
            kv_acc[g] += _mm(_unpack(pkt_s[g]), vbs[g])

    def a1_q(i, xn, gs=range(G), after=None):
        for n, g in enumerate(gs):
            q = _mm(xn, wa_qkv[:, _gs(g)])
            pq_s[prows_of(i), _gs(g)] = _pack(_phi(q))
            if after is not None:
                after(n, q)

    def a_reset():
        kv_acc[...] = jnp.zeros(kv_acc.shape, F32)
        z_acc[...] = jnp.zeros(z_acc.shape, F32)

    def a_fin_z():
        zr = lax.broadcasted_iota(jnp.int32, (16, 128), 0)
        zc = lax.broadcasted_iota(jnp.int32, (16, 128), 1) // DH
        z = jnp.sum(z_acc[...], axis=0, keepdims=True)
        for g in range(G):
            zt_s[g] = _pack(jnp.where(zr == zc, z[:, _gs(g)], 0.0))

    def a_fin_m():
        r = lax.broadcasted_iota(jnp.int32, (128, 128), 0) // DH
        c = lax.broadcasted_iota(jnp.int32, (128, 128), 1) // DH
        same = r == c
        for g in range(G):
            kvm = jnp.where(same, kv_acc[g], 0.0).astype(BF16)
            m_s[g * 64:(g + 1) * 64, :] = _pack(_mm(kvm, wa_o[_gs(g), :]))

    def a2_pqn(i, g):
        pq = _unpack(pq_s[prows_of(i), _gs(g)])
        dent = lax.dot_general(_unpack(zt_s[g]), pq, NT_DIMS, preferred_element_type=F32)
        r = _recip(dent[0:8] + 1e-6)
        rb = jnp.concatenate(
            [jnp.broadcast_to(r[u:u + 1], (DH, TM)) for u in range(HPG)], axis=0)
        return (pq.astype(F32) * rb.T).astype(BF16)

    def b1_v(i, xn, g):
        w = _unpack(w0_s[1]) if g == 0 else wb_qkv[:, 2 * D + g * 128:2 * D + (g + 1) * 128]
        v = _mm(xn, w)
        vt_s[g * 64:(g + 1) * 64, rows_of(i)] = _pack(v.T)
        return v

    def b1_q(i, xn, after=None):
        for g in range(G):
            q = _mm(xn, wb_qkv[:, _gs(g)])
            qt_s[g * 64:(g + 1) * 64, rows_of(i)] = _pack((q * QSCALE).T)
            if after is not None:
                after(g, q)

    def b1_k(i, xn, after=None):
        for g in range(G):
            k = _mm(xn, wb_qkv[:, D + g * 128:D + (g + 1) * 128])
            k_s[g, prows_of(i), :] = _pack(k)
            if after is not None:
                after(g, k)

    def kb_maker(g, flag, nslots):
        k32 = k_s[g, 0:NOFF // 2, :]
        state = {"slot": 0}

        def step(tok):
            s = state["slot"]
            state["slot"] += 1
            if s >= nslots:
                return
            kk = jnp.where(flag, pltpu.bitcast(tok[0:NOFF // 2], U32), k32)
            kk = _unpack(kk).astype(F32)
            for d in range((s * 128) // nslots, ((s + 1) * 128) // nslots):
                kb_s[g, d] = jnp.broadcast_to(kk[:, d:d + 1], (NOFF, 128))

        return step

    def attn_group(ja, jb, flag, extra=None):
        outs = []
        sa = {}
        sb = {"acc": None}
        nunits = (NOFF // 16) * DH
        for kind, idx in _attn_order():
            v, c = divmod(idx, NC)
            t, u = divmod(v, HPG)
            ks = slice(c * TK, (c + 1) * TK)
            if kind == "b" and jb is not None:
                if c == 0:
                    prev = sb["acc"]
                    sb = dict(hrows=_ds((jb // SPG) * 64 + u * (DH // 2), DH // 2),
                              m8=m_buf[v], lrun=None,
                              acc=None if prev is None else jnp.where(flag, prev, 0.0))
                p = jnp.exp2(s_buf[v, ks, :].reshape(TK // 8, 8, TQ) - sb["m8"][None]).reshape(TK, TQ)
                lrun = sb["lrun"]
                for r in reversed(range(TK // 16)):
                    pr = p[16 * r:16 * r + 8] + p[16 * r + 8:16 * r + 16]
                    lrun = pr if lrun is None else lrun + pr
                sb["lrun"] = lrun
                ot = _mm(_unpack(vt_s[sb["hrows"], ks]), p.astype(BF16))
                sb["acc"] = ot if sb["acc"] is None else sb["acc"] + ot
                if c == NC - 1:
                    l = jnp.sum(lrun, axis=0, keepdims=True)
                    outs.append(sb["acc"] * (1.0 / l))
                    if u == HPG - 1:
                        ot = jnp.concatenate(outs, axis=0)
                        outs = []
                        qt = (jb % SPG) * QPS + t
                        o_s[_ds(qt * (TQ // 2), TQ // 2), _ds((jb // SPG) * 128, 128)] = _pack(ot.T)
            if kind == "a" and extra is not None:
                extra(idx)
            if kind == "a" and ja is not None:
                if c == 0:
                    ga = ja // SPG
                    qt = (ja % SPG) * QPS + t
                    qh = _unpack(qt_s[_ds(ga * 64 + u * (DH // 2), DH // 2), _ds(qt * TQ, TQ)])
                    qf = qh.astype(F32)
                    for d in range(DH):
                        qb_s[u, d] = jnp.broadcast_to(qf[d:d + 1], (8, TQ))
                    parts = []
                    if u > 0:
                        parts.append(jnp.zeros((u * DH, TQ), BF16))
                    parts.append(qh)
                    if u < HPG - 1:
                        parts.append(jnp.zeros(((HPG - 1 - u) * DH, TQ), BF16))
                    sa = dict(qm=jnp.concatenate(parts, axis=0), g=ga, mrun=None, nt=0, unit=0, sv=None)
                r0, nm = _a_chunks(v == 0)[c]
                kc = _unpack(k_s[sa["g"], r0 // 2:(r0 + nm) // 2, :])
                st = _mm(kc, sa["qm"])
                s_buf[v, r0:r0 + nm, :] = st
                mc = jnp.max(st.reshape(nm // 8, 8, TQ), axis=0)
                for r in range(nm // 16):
                    sa["nt"] += 1
                    upto = min(nunits, (sa["nt"] * nunits + VSPAN - 1) // VSPAN)
                    while sa["unit"] < upto:
                        tok = st[16 * r:16 * r + 8, 0:128]
                        blk, d = divmod(sa["unit"], DH)
                        kb = kb_s[sa["g"], u * DH + d, blk * 16:(blk + 1) * 16, :]
                        k0, k1 = kb[0:8], kb[8:16]
                        if d % 2 == 0:
                            k0 = jnp.where(flag, tok, k0)
                        else:
                            k1 = jnp.where(flag, tok, k1)
                        qb = qb_s[u, d]
                        tt = jnp.concatenate(
                            [jnp.concatenate([k0] * (TQ // 128), axis=1) * qb,
                             jnp.concatenate([k1] * (TQ // 128), axis=1) * qb], axis=0)
                        sa["sv"] = tt if d == 0 else sa["sv"] + tt
                        if d == DH - 1:
                            sv = sa["sv"]
                            s_buf[v, blk * 16:(blk + 1) * 16, :] = sv
                            mc = jnp.maximum(mc, jnp.maximum(sv[0:8], sv[8:16]))
                        sa["unit"] += 1
                sa["mrun"] = mc if sa["mrun"] is None else jnp.maximum(sa["mrun"], mc)
                if c == NC - 1:
                    assert sa["unit"] == nunits
                    m_buf[v] = jnp.broadcast_to(jnp.max(sa["mrun"], axis=0, keepdims=True), (8, TQ))

    def attn_loop():
        def body(j, carry):
            attn_group(j + 1, j, j < 0)
            return carry

        lax.fori_loop(0, NSTEP - 1, body, 0)

    def tile_mm_pieces(lhs_of, w_ref, col0, init_of, done):
        part = []
        nk = D // PK

        def piece(r):
            n, kh = divmod(r, nk)
            kk = slice(kh * PK, (kh + 1) * PK)
            y = _mm(lhs_of(kk), w_ref[kk, col0 + n * 128:col0 + (n + 1) * 128])
            if kh == 0:
                part.append(init_of(n) + y)
            elif kh < nk - 1:
                part.append(part.pop() + y)
            else:
                done(n, part.pop() + y)

        return piece

    def b3_pieces(i, finish, after=None):
        cols = []

        def done(n, y):
            cols.append(y)
            if after is not None:
                after(n, y)
            if n == G - 1:
                finish(jnp.concatenate(cols, axis=1))

        return tile_mm_pieces(lambda kk: _unpack(o_s[prows_of(i), kk]), wb_o, 0,
                              lambda n: x_s[rows_of(i), _gs(n)], done)

    def attn_tail_final():
        def finish(i):
            def f(x):
                xio_s[rows_of(i), :] = x.astype(BF16)
            return f

        parts = [b3_pieces(i, finish(i)) for i in range(2 * QPS)]
        attn_group(None, NSTEP - 1, flag_s[0] != 0, lambda idx: parts[idx // 32](idx % 32))

    def attn_tail_mid():
        flag = flag_s[0] != 0
        lns = {}
        pkts = []
        vbs = []

        def finish(i):
            def f(x):
                x_s[rows_of(i), :] = x
                lns[i] = ln_after(i, x, flag, 2)
            return f

        def k_done(n, k):
            lns[1](n, k)
            pkts.append(a1_k_post(k, n))

        xn0_val = []

        def xn0(kk):
            if not xn0_val:
                xn0_val.append(xn_of(0))
            return xn0_val[0][:, kk]

        def zero(n):
            return jnp.where(flag, x_s[rows_of(2), _gs(n)], 0.0)

        parts = [
            b3_pieces(0, finish(0)),
            b3_pieces(1, finish(1), lambda n, y: lns[0](n, y)),
            tile_mm_pieces(xn0, wa_qkv, D, zero, k_done),
            tile_mm_pieces(xn0, wa_qkv, 2 * D, zero, lambda n, v: vbs.append(v.astype(BF16))),
        ]
        attn_group(None, NSTEP - 1, flag, lambda idx: parts[idx // 32](idx % 32))
        a1_k_store(xn_of(1))
        for g in range(G):
            kv_acc[g] += _mm(pkts[g], vbs[g])
        a1_q(0, xn0_val[0])

    def a1_last_and_a2_first(src):
        i = NTM - 1
        xn = xn_of(i)
        a_fin_z()
        a1_v(xn)
        pqn = []
        for g in range(G // 2):
            a1_q(i, xn, [g])
            pqn.append(a2_pqn(0, 2 * g))
            pqn.append(a2_pqn(0, 2 * g + 1))
        a_fin_m()
        x = resid(0, jnp.concatenate(pqn, axis=1), _unpack(m_s[...]), src)
        a1_q(i, xn, range(G // 2, G), ln_after(0, x, flag_s[0] != 0, 3))
        b1_k(0, xn_of(0))

    def a2b1_body(src, i, carry):
        flag = i < 0
        xn = xn_of(i)
        kb_step = kb_maker(i, flag, KB_SLOTS)
        pqn = []
        for g in range(G):
            kb_step(b1_v(i, xn, g))
            for _ in range(DEN_SCHED[g]):
                pqn.append(a2_pqn(i + 1, len(pqn)))
        x = resid(i + 1, jnp.concatenate(pqn, axis=1), _unpack(m_s[...]), src)
        for g in range(G):
            kb_step(x[:, _gs(g)])
        ln = ln_after(i + 1, x, flag, 2)

        def after_q(g, q):
            ln(g, q)
            if g >= G // 2:
                kb_step(q)

        b1_q(i, xn, after_q)
        b1_k(i + 1, xn_of(i + 1), lambda g, k: kb_step(k))
        return carry

    def b1_last_and_attn():
        i = NTM - 1
        flag = flag_s[0] != 0
        xn = xn_of(i)
        kb_step = kb_maker(G - 1, flag, 16)
        for g in range(G):
            kb_step(b1_v(i, xn, g))
        b1_q(i, xn, lambda g, q: kb_step(q))
        attn_group(0, None, flag)

    def b3a1_body(i, carry):
        xn = xn_of(i)
        x = resid(i + 1, _unpack(o_s[prows_of(i + 1), :]), wb_o_full(), x_s)
        a1_v(xn, ln_after(i + 1, x, i < 0, 2))
        a1_k_store(xn_of(i + 1))
        a1_q(i, xn)
        return carry

    def a1_first_body(i, carry):
        cp_x(i + 1).wait()
        xn = xn_of(i)
        x = xio_s[rows_of(i + 1), :].astype(F32)
        a1_v(xn, ln_after(i + 1, x, i < 0, 2))
        a1_k_store(xn_of(i + 1))
        a1_q(i, xn)
        return carry

    def b3out(r0, nr):
        rows = pl.ds(r0, nr)
        x = x_s[rows, :] + _mm(_unpack(o_s[pl.ds(r0 // 2, nr // 2), :]), wb_o[...])
        xio_s[rows, :] = x.astype(BF16)

    flag_s[0] = 0
    cp_x(0).start()
    cp_wak0.start()
    a_reset()
    cp_x(0).wait()
    cp_x(1).start()
    ln_in(0)
    cp_wak0.wait()
    cp_wak1.start()
    xn = xn_of(0)
    pkts = a1_k(xn, [0])
    k = k_raw(xn, 1)
    cp_x(1).wait()
    pkts.append(a1_k_post(k, 1))
    ln_in(1)
    pkts += a1_k(xn, [2, 3])
    xn1 = xn_of(1)
    for g in range(3):
        pkt_s[g] = _pack(a1_k(xn1, [g])[0])
        if g == 0:
            cp_wav.start()
    k = k_raw(xn1, 3)
    cp_wak1.wait()
    pkt_s[3] = _pack(a1_k_post(k, 3))
    pkts += a1_k(xn, range(G // 2, G))
    for g in range(G // 2, G - 1):
        pkt_s[g] = _pack(a1_k(xn1, [g])[0])
        if g == G // 2:
            cp_waq.start()
    k = k_raw(xn1, G - 1)
    cp_wav.wait()
    cp_x(2).start()
    pkt_s[G - 1] = _pack(a1_k_post(k, G - 1))
    w0_s[0] = _pack(wa_qkv[:, 2 * D:2 * D + 128])
    vbs = [_mm(xn, wa_qkv[:, 2 * D + g * 128:2 * D + (g + 1) * 128]).astype(BF16) for g in range(G)]
    cp_waq.wait()
    for i in range(3, NTM):
        cp_x(i).start()
    a1_q(0, xn, range(2))
    for g in range(G):
        kv_acc[g] += _mm(pkts[g], vbs[g])
    a1_q(0, xn, range(2, G))
    cp_wao.start()
    cp_wbq.start()
    cp_wbo.start()
    lax.fori_loop(1, NTM - 1, a1_first_body, 0)
    cp_wao.wait()
    cp_wbq.wait()
    cp_wbo.wait()
    w0_s[1] = _pack(wb_qkv[:, 2 * D:2 * D + 128])
    w0_s[2] = _pack(wb_o[:, 0:128])

    for l in range(2):
        src = xio_s if l == 0 else x_s
        a1_last_and_a2_first(src)
        lax.fori_loop(0, NTM - 1, functools.partial(a2b1_body, src), 0)
        b1_last_and_attn()
        attn_loop()
        if l == 0:
            a_reset()
            attn_tail_mid()
            lax.fori_loop(1, NTM - 1, b3a1_body, 0)
        else:
            attn_tail_final()
            for i in range(2 * QPS):
                cp_out(i).start()
            for i in range(2 * QPS, NTM - 1):
                b3out(i * TM, TM)
                cp_out(i).start()
            for h in range(2):
                b3out(S - TM + h * (TM // 2), TM // 2)
                cp_last(h).start()
    for i in range(NTM - 1):
        cp_out(i).wait()
    for h in range(2):
        cp_last(h).wait()


@jax.jit
def pallas_interleave_layers__linear_attn_block__mha_block__prompt_kernel(
    A_x: jax.Array,
    A_wqkv: jax.Array,
    A_wo: jax.Array,
    B_x: jax.Array,
    B_wqkv: jax.Array,
    B_wo: jax.Array,
):
    del B_x
    x = A_x.reshape(S, D)
    any_spec = pl.BlockSpec(memory_space=pl.ANY)
    out = pl.pallas_call(
        _kernel,
        out_shape=jax.ShapeDtypeStruct((S, D), BF16),
        in_specs=[any_spec] * 5,
        out_specs=any_spec,
        scratch_shapes=[
            pltpu.VMEM((S, D), BF16),
            pltpu.VMEM((S, D), F32),
            pltpu.VMEM((TM // 2, D), U32),
            pltpu.VMEM((D, 3 * D), BF16),
            pltpu.VMEM((D, D), BF16),
            pltpu.VMEM((D, 3 * D), BF16),
            pltpu.VMEM((D, D), BF16),
            pltpu.VMEM((S // 2, D), U32),
            pltpu.VMEM((G, 64, TM), U32),
            pltpu.VMEM((D // 2, S), U32),
            pltpu.VMEM((G, S // 2, 128), U32),
            pltpu.VMEM((D // 2, S), U32),
            pltpu.VMEM((G, 128, 128), F32),
            pltpu.VMEM((8, D), F32),
            pltpu.VMEM((G, 8, 128), U32),
            pltpu.VMEM((D // 2, D), U32),
            pltpu.VMEM((NV, S, TQ), F32),
            pltpu.VMEM((NV, 8, TQ), F32),
            pltpu.VMEM((HPG, DH, 8, TQ), F32),
            pltpu.VMEM((G, 128, NOFF, 128), F32),
            pltpu.VMEM((3, D // 2, 128), U32),
            pltpu.SMEM((1,), jnp.int32),
            pltpu.SemaphoreType.DMA((NTM + 1,)),
            pltpu.SemaphoreType.DMA((7,)),
        ],
        compiler_params=pltpu.CompilerParams(vmem_limit_bytes=128 * 1024 * 1024),
    )(x, A_wqkv, A_wo, B_wqkv, B_wo)
    return out.reshape(1, S, D)
```

```python
import functools
import math

import jax
import jax.numpy as jnp
from jax import lax
import jax.experimental.pallas as pl
import jax.experimental.pallas.tpu as pltpu

S = 2048
D = 1024
H = 32
DH = D // H
G = D // 128
HPG = 128 // DH
TM = 256
NTM = S // TM
RC = 32
NRC = TM // RC
TQ = 512
TK = 128
NQ = S // TQ
NC = S // TK
QPS = 2
NV = QPS * HPG
SPG = NQ // QPS
NSTEP = G * SPG
LEAD_AT = 4
NOFF = 64
VSPAN = 120
KB_SLOTS = 26
PK = 256
DEN_SCHED = (2, 1, 2, 1, 1, 1, 0, 0)

F32 = jnp.float32
BF16 = jnp.bfloat16
U32 = jnp.uint32
NT_DIMS = (((1,), (1,)), ((), ()))
QSCALE = (DH ** -0.5) * math.log2(math.e)


def _recip(d):
    r = pl.reciprocal(d, approx=True)
    return r * (2.0 - d * r)


def _layernorm(x, tok=None, flag=None):
    m = jnp.mean(x, axis=-1, keepdims=True)
    if tok is not None:
        m = jnp.where(flag, tok, m)
    xc = x - m
    v = jnp.mean(xc * xc, axis=-1, keepdims=True)
    return xc * lax.rsqrt(v + 1e-5)


def _phi(t):
    return jnp.where(t > 0, t + 1.0, jnp.exp(t)) + 1e-6


def _mm(a, b):
    return jnp.dot(a, b, preferred_element_type=F32)


def _gs(g):
    return slice(g * 128, (g + 1) * 128)


def _ds(start, size, mult=None):
    if isinstance(start, int):
        return pl.ds(start, size)
    return pl.ds(pl.multiple_of(start, mult or size), size)


def _pack(x):
    return pltpu.bitcast(x.astype(BF16), U32)


def _unpack(x):
    return pltpu.bitcast(x, BF16)


def _a_chunks(first):
    if first:
        sizes = [TK - NOFF] + [TK] * (NC - 1)
    else:
        sizes = [TK] * NC
        n = NOFF // 16
        for i in range(n):
            sizes[(i * NC) // n + 1] -= 16
    return [(NOFF + sum(sizes[:i]), sizes[i]) for i in range(NC)]


def _attn_order():
    n = NV * NC
    order = []
    bi = ai = 0
    while ai < n:
        if bi < n:
            order.append(("b", bi))
            bi += 1
            if ai == LEAD_AT:
                order.append(("b", bi))
                bi += 1
        order.append(("a", ai))
        ai += 1
    return order


def _kernel(x_hbm, wa_qkv_hbm, wa_o_hbm, wb_qkv_hbm, wb_o_hbm, out_hbm,
            xio_s, x_s, xn_s, wa_qkv, wa_o, wb_qkv, wb_o,
            pq_s, pkt_s, qt_s, k_s, vt_s, kv_acc, z_acc, zt_s, m_s, s_buf, m_buf, qb_s, kb_s, w0_s,
            flag_s, x_sems, w_sems):
    o_s = pq_s

    def rows_of(i):
        return _ds(i * TM, TM)

    def prows_of(i):
        return _ds(i * (TM // 2), TM // 2)

    def cp_x(i):
        return pltpu.make_async_copy(x_hbm.at[rows_of(i)], xio_s.at[rows_of(i)], x_sems.at[i])

    def cp_out(i):
        return pltpu.make_async_copy(xio_s.at[rows_of(i)], out_hbm.at[rows_of(i)], x_sems.at[i])

    def cp_last(h):
        rows = pl.ds(S - TM + h * (TM // 2), TM // 2)
        return pltpu.make_async_copy(xio_s.at[rows], out_hbm.at[rows], x_sems.at[NTM - 1 + h])

    def cp_wa(col0, ncol, sem):
        cols = pl.ds(col0, ncol)
        return pltpu.make_async_copy(wa_qkv_hbm.at[:, cols], wa_qkv.at[:, cols], w_sems.at[sem])

    cp_waq = cp_wa(0, D, 0)
    cp_wak0 = cp_wa(D, D // 2, 1)
    cp_wak1 = cp_wa(D + D // 2, D // 2, 6)
    cp_wav = cp_wa(2 * D, D, 2)
    cp_wao = pltpu.make_async_copy(wa_o_hbm, wa_o, w_sems.at[3])
    cp_wbq = pltpu.make_async_copy(wb_qkv_hbm, wb_qkv, w_sems.at[4])
    cp_wbo = pltpu.make_async_copy(wb_o_hbm, wb_o, w_sems.at[5])

    def xn_of(i):
        del i
        return _unpack(xn_s[...])

    def ln_in(i):
        x = xio_s[rows_of(i), :].astype(F32)
        xn_s[...] = _pack(_layernorm(x))

    def ln_after(i, x, flag, per):
        def after(n, tok):
            for r in range(n * per, min((n + 1) * per, NRC)):
                xr = x[r * RC:(r + 1) * RC]
                xn_s[pl.ds(r * (RC // 2), RC // 2), :] = _pack(
                    _layernorm(xr, tok[0:RC, 0:1], flag))
        return after

    def resid(i, o, w, src):
        rows = rows_of(i)
        x = src[rows, :].astype(F32) + _mm(o, w)
        x_s[rows, :] = x
        return x

    def wb_o_full():
        return jnp.concatenate([_unpack(w0_s[2]), wb_o[:, 128:D]], axis=1)

    def a1_k_post(k, g):
        pk = _phi(k)
        z_acc[:, _gs(g)] += jnp.sum(pk.reshape(pk.shape[0] // 8, 8, 128), axis=0)
        return pk.T.astype(BF16)

    def k_raw(xn, g):
        return _mm(xn, wa_qkv[:, D + g * 128:D + (g + 1) * 128])

    def a1_k(xn, gs=range(G)):
        return [a1_k_post(k_raw(xn, g), g) for g in gs]

    def a1_k_store(xn):
        for g, pkt in enumerate(a1_k(xn)):
            pkt_s[g] = _pack(pkt)

    def a1_v(xn, after=None):
        vbs = []
        for g in range(G):
            w = _unpack(w0_s[0]) if g == 0 else wa_qkv[:, 2 * D + g * 128:2 * D + (g + 1) * 128]
            v = _mm(xn, w)
            vbs.append(v.astype(BF16))
            if after is not None:
                after(g, v)
        for g in range(G):
            kv_acc[g] += _mm(_unpack(pkt_s[g]), vbs[g])

    def a1_q(i, xn, gs=range(G), after=None):
        for n, g in enumerate(gs):
            q = _mm(xn, wa_qkv[:, _gs(g)])
            pq_s[prows_of(i), _gs(g)] = _pack(_phi(q))
            if after is not None:
                after(n, q)

    def a_reset():
        kv_acc[...] = jnp.zeros(kv_acc.shape, F32)
        z_acc[...] = jnp.zeros(z_acc.shape, F32)

    def a_fin_z():
        zr = lax.broadcasted_iota(jnp.int32, (16, 128), 0)
        zc = lax.broadcasted_iota(jnp.int32, (16, 128), 1) // DH
        z = jnp.sum(z_acc[...], axis=0, keepdims=True)
        for g in range(G):
            zt_s[g] = _pack(jnp.where(zr == zc, z[:, _gs(g)], 0.0))

    def a_fin_m():
        r = lax.broadcasted_iota(jnp.int32, (128, 128), 0) // DH
        c = lax.broadcasted_iota(jnp.int32, (128, 128), 1) // DH
        same = r == c
        for g in range(G):
            kvm = jnp.where(same, kv_acc[g], 0.0).astype(BF16)
            m_s[g * 64:(g + 1) * 64, :] = _pack(_mm(kvm, wa_o[_gs(g), :]))

    def a2_pqn(i, g):
        pq = _unpack(pq_s[prows_of(i), _gs(g)])
        dent = lax.dot_general(_unpack(zt_s[g]), pq, NT_DIMS, preferred_element_type=F32)
        r = _recip(dent[0:8] + 1e-6)
        rb = jnp.concatenate(
            [jnp.broadcast_to(r[u:u + 1], (DH, TM)) for u in range(HPG)], axis=0)
        return (pq.astype(F32) * rb.T).astype(BF16)

    def b1_v(i, xn, g):
        w = _unpack(w0_s[1]) if g == 0 else wb_qkv[:, 2 * D + g * 128:2 * D + (g + 1) * 128]
        v = _mm(xn, w)
        vt_s[g * 64:(g + 1) * 64, rows_of(i)] = _pack(v.T)
        return v

    def b1_q(i, xn, after=None):
        for g in range(G):
            q = _mm(xn, wb_qkv[:, _gs(g)])
            qt_s[g * 64:(g + 1) * 64, rows_of(i)] = _pack((q * QSCALE).T)
            if after is not None:
                after(g, q)

    def b1_k(i, xn, after=None):
        for g in range(G):
            k = _mm(xn, wb_qkv[:, D + g * 128:D + (g + 1) * 128])
            k_s[g, prows_of(i), :] = _pack(k)
            if after is not None:
                after(g, k)

    def kb_maker(g, flag, nslots):
        k32 = k_s[g, 0:NOFF // 2, :]
        state = {"slot": 0}

        def step(tok):
            s = state["slot"]
            state["slot"] += 1
            if s >= nslots:
                return
            kk = jnp.where(flag, pltpu.bitcast(tok[0:NOFF // 2], U32), k32)
            kk = _unpack(kk).astype(F32)
            for d in range((s * 128) // nslots, ((s + 1) * 128) // nslots):
                kb_s[g, d] = jnp.broadcast_to(kk[:, d:d + 1], (NOFF, 128))

        return step

    def attn_group(ja, jb, flag, extra=None):
        outs = []
        sa = {}
        sb = {"acc": None}
        nunits = (NOFF // 16) * DH
        for kind, idx in _attn_order():
            v, c = divmod(idx, NC)
            t, u = divmod(v, HPG)
            ks = slice(c * TK, (c + 1) * TK)
            if kind == "b" and jb is not None:
                if c == 0:
                    prev = sb["acc"]
                    m8 = m_buf[v]
                    if v == NV - 1:
                        m8 = jnp.broadcast_to(jnp.max(m8, axis=0, keepdims=True), (8, TQ))
                    sb = dict(hrows=_ds((jb // SPG) * 64 + u * (DH // 2), DH // 2),
                              m8=m8, lrun=None,
                              acc=None if prev is None else jnp.where(flag, prev, 0.0))
                p = jnp.exp2(s_buf[v, ks, :].reshape(TK // 8, 8, TQ) - sb["m8"][None]).reshape(TK, TQ)
                lrun = sb["lrun"]
                for r in reversed(range(TK // 16)):
                    pr = p[16 * r:16 * r + 8] + p[16 * r + 8:16 * r + 16]
                    lrun = pr if lrun is None else lrun + pr
                sb["lrun"] = lrun
                ot = _mm(_unpack(vt_s[sb["hrows"], ks]), p.astype(BF16))
                sb["acc"] = ot if sb["acc"] is None else sb["acc"] + ot
                if c == NC - 1:
                    l = jnp.sum(lrun, axis=0, keepdims=True)
                    outs.append(sb["acc"] * (1.0 / l))
                    if u == HPG - 1:
                        ot = jnp.concatenate(outs, axis=0)
                        outs = []
                        qt = (jb % SPG) * QPS + t
                        o_s[_ds(qt * (TQ // 2), TQ // 2), _ds((jb // SPG) * 128, 128)] = _pack(ot.T)
            if kind == "a" and extra is not None:
                extra(idx)
            if kind == "a" and ja is not None:
                if c == 0:
                    ga = ja // SPG
                    qt = (ja % SPG) * QPS + t
                    qh = _unpack(qt_s[_ds(ga * 64 + u * (DH // 2), DH // 2), _ds(qt * TQ, TQ)])
                    qf = qh.astype(F32)
                    for d in range(DH):
                        qb_s[u, d] = jnp.broadcast_to(qf[d:d + 1], (8, TQ))
                    parts = []
                    if u > 0:
                        parts.append(jnp.zeros((u * DH, TQ), BF16))
                    parts.append(qh)
                    if u < HPG - 1:
                        parts.append(jnp.zeros(((HPG - 1 - u) * DH, TQ), BF16))
                    sa = dict(qm=jnp.concatenate(parts, axis=0), g=ga, mrun=None, nt=0, unit=0, sv=None)
                r0, nm = _a_chunks(v == 0)[c]
                kc = _unpack(k_s[sa["g"], r0 // 2:(r0 + nm) // 2, :])
                st = _mm(kc, sa["qm"])
                s_buf[v, r0:r0 + nm, :] = st
                mc = jnp.max(st.reshape(nm // 8, 8, TQ), axis=0)
                for r in range(nm // 16):
                    sa["nt"] += 1
                    upto = min(nunits, (sa["nt"] * nunits + VSPAN - 1) // VSPAN)
                    while sa["unit"] < upto:
                        tok = st[16 * r:16 * r + 8, 0:128]
                        blk, d = divmod(sa["unit"], DH)
                        kb = kb_s[sa["g"], u * DH + d, blk * 16:(blk + 1) * 16, :]
                        k0, k1 = kb[0:8], kb[8:16]
                        if d % 2 == 0:
                            k0 = jnp.where(flag, tok, k0)
                        else:
                            k1 = jnp.where(flag, tok, k1)
                        qb = qb_s[u, d]
                        tt = jnp.concatenate(
                            [jnp.concatenate([k0] * (TQ // 128), axis=1) * qb,
                             jnp.concatenate([k1] * (TQ // 128), axis=1) * qb], axis=0)
                        sa["sv"] = tt if d == 0 else sa["sv"] + tt
                        if d == DH - 1:
                            sv = sa["sv"]
                            s_buf[v, blk * 16:(blk + 1) * 16, :] = sv
                            mc = jnp.maximum(mc, jnp.maximum(sv[0:8], sv[8:16]))
                        sa["unit"] += 1
                sa["mrun"] = mc if sa["mrun"] is None else jnp.maximum(sa["mrun"], mc)
                if c == NC - 1:
                    assert sa["unit"] == nunits
                    if v == NV - 1:
                        m_buf[v] = sa["mrun"]
                    else:
                        m_buf[v] = jnp.broadcast_to(jnp.max(sa["mrun"], axis=0, keepdims=True), (8, TQ))

    def attn_loop():
        def body(j, carry):
            attn_group(j + 1, j, j < 0)
            return carry

        lax.fori_loop(0, NSTEP - 1, body, 0)

    def tile_mm_pieces(lhs_of, w_ref, col0, init_of, done):
        part = []
        nk = D // PK

        def piece(r):
            n, kh = divmod(r, nk)
            kk = slice(kh * PK, (kh + 1) * PK)
            y = _mm(lhs_of(kk), w_ref[kk, col0 + n * 128:col0 + (n + 1) * 128])
            if kh == 0:
                part.append(init_of(n) + y)
            elif kh < nk - 1:
                part.append(part.pop() + y)
            else:
                done(n, part.pop() + y)

        return piece

    def b3_pieces(i, finish, after=None):
        cols = []

        def done(n, y):
            cols.append(y)
            if after is not None:
                after(n, y)
            if n == G - 1:
                finish(jnp.concatenate(cols, axis=1))

        return tile_mm_pieces(lambda kk: _unpack(o_s[prows_of(i), kk]), wb_o, 0,
                              lambda n: x_s[rows_of(i), _gs(n)], done)

    def attn_tail_final():
        def finish(i):
            def f(x):
                xio_s[rows_of(i), :] = x.astype(BF16)
            return f

        parts = [b3_pieces(i, finish(i)) for i in range(2 * QPS)]
        attn_group(None, NSTEP - 1, flag_s[0] != 0, lambda idx: parts[idx // 32](idx % 32))

    def attn_tail_mid():
        flag = flag_s[0] != 0
        lns = {}
        pkts = []
        vbs = []

        def finish(i):
            def f(x):
                x_s[rows_of(i), :] = x
                lns[i] = ln_after(i, x, flag, 2)
            return f

        def k_done(n, k):
            pkts.append(a1_k_post(k, n))

        def v_done(n, v):
            lns[1](n, v)
            vbs.append(v.astype(BF16))

        xn0_val = []

        def xn0(kk):
            if not xn0_val:
                xn0_val.append(xn_of(0))
            return xn0_val[0][:, kk]

        def zero(n):
            return jnp.where(flag, x_s[rows_of(2), _gs(n)], 0.0)

        parts = [
            b3_pieces(0, finish(0)),
            b3_pieces(1, finish(1), lambda n, y: lns[0](n, y)),
            tile_mm_pieces(xn0, wa_qkv, D, zero, k_done),
            tile_mm_pieces(xn0, wa_qkv, 2 * D, zero, v_done),
        ]
        attn_group(None, NSTEP - 1, flag, lambda idx: parts[idx // 32](idx % 32))
        a1_k_store(xn_of(1))
        for g in range(G):
            kv_acc[g] += _mm(pkts[g], vbs[g])
        a1_q(0, xn0_val[0])

    def a1_last_and_a2_first(src):
        i = NTM - 1
        xn = xn_of(i)
        a_fin_z()
        a1_v(xn)
        pqn = []
        for g in range(G // 2):
            a1_q(i, xn, [g])
            pqn.append(a2_pqn(0, 2 * g))
            pqn.append(a2_pqn(0, 2 * g + 1))
        a_fin_m()
        x = resid(0, jnp.concatenate(pqn, axis=1), _unpack(m_s[...]), src)
        a1_q(i, xn, range(G // 2, G), ln_after(0, x, flag_s[0] != 0, 3))
        b1_k(0, xn_of(0))

    def a2b1_body(src, i, carry):
        flag = i < 0
        xn = xn_of(i)
        kb_step = kb_maker(i, flag, KB_SLOTS)
        pqn = []
        for g in range(G):
            kb_step(b1_v(i, xn, g))
            for _ in range(DEN_SCHED[g]):
                pqn.append(a2_pqn(i + 1, len(pqn)))
        x = resid(i + 1, jnp.concatenate(pqn, axis=1), _unpack(m_s[...]), src)
        for g in range(G):
            kb_step(x[:, _gs(g)])
        ln = ln_after(i + 1, x, flag, 2)

        def after_q(g, q):
            ln(g, q)
            if g >= G // 2:
                kb_step(q)

        b1_q(i, xn, after_q)
        b1_k(i + 1, xn_of(i + 1), lambda g, k: kb_step(k))
        return carry

    def b1_last_and_attn():
        i = NTM - 1
        flag = flag_s[0] != 0
        xn = xn_of(i)
        kb_step = kb_maker(G - 1, flag, 16)
        for g in range(G):
            kb_step(b1_v(i, xn, g))
        b1_q(i, xn, lambda g, q: kb_step(q))
        attn_group(0, None, flag)

    def b3a1_body(i, carry):
        xn = xn_of(i)
        x = resid(i + 1, _unpack(o_s[prows_of(i + 1), :]), wb_o_full(), x_s)
        a1_v(xn, ln_after(i + 1, x, i < 0, 2))
        a1_k_store(xn_of(i + 1))
        a1_q(i, xn)
        return carry

    def a1_first_body(i, carry):
        cp_x(i + 1).wait()
        xn = xn_of(i)
        x = xio_s[rows_of(i + 1), :].astype(F32)
        a1_v(xn, ln_after(i + 1, x, i < 0, 2))
        a1_k_store(xn_of(i + 1))
        a1_q(i, xn)
        return carry

    def b3out(r0, nr):
        rows = pl.ds(r0, nr)
        x = x_s[rows, :] + _mm(_unpack(o_s[pl.ds(r0 // 2, nr // 2), :]), wb_o[...])
        xio_s[rows, :] = x.astype(BF16)

    flag_s[0] = 0
    cp_x(0).start()
    cp_wak0.start()
    a_reset()
    cp_x(0).wait()
    cp_x(1).start()
    ln_in(0)
    cp_wak0.wait()
    cp_wak1.start()
    xn = xn_of(0)
    pkts = a1_k(xn, [0])
    k = k_raw(xn, 1)
    cp_x(1).wait()
    pkts.append(a1_k_post(k, 1))
    ln_in(1)
    pkts += a1_k(xn, [2, 3])
    xn1 = xn_of(1)
    for g in range(3):
        pkt_s[g] = _pack(a1_k(xn1, [g])[0])
        if g == 0:
            cp_wav.start()
    k = k_raw(xn1, 3)
    cp_wak1.wait()
    pkt_s[3] = _pack(a1_k_post(k, 3))
    pkts += a1_k(xn, range(G // 2, G))
    for g in range(G // 2, G - 1):
        pkt_s[g] = _pack(a1_k(xn1, [g])[0])
        if g == G // 2:
            cp_waq.start()
    k = k_raw(xn1, G - 1)
    cp_wav.wait()
    cp_x(2).start()
    pkt_s[G - 1] = _pack(a1_k_post(k, G - 1))
    w0_s[0] = _pack(wa_qkv[:, 2 * D:2 * D + 128])
    vbs = [_mm(xn, wa_qkv[:, 2 * D + g * 128:2 * D + (g + 1) * 128]).astype(BF16) for g in range(G)]
    cp_waq.wait()
    for i in range(3, NTM):
        cp_x(i).start()
    a1_q(0, xn, range(2))
    for g in range(G):
        kv_acc[g] += _mm(pkts[g], vbs[g])
    a1_q(0, xn, range(2, G))
    cp_wao.start()
    cp_wbq.start()
    cp_wbo.start()
    lax.fori_loop(1, NTM - 1, a1_first_body, 0)
    cp_wao.wait()
    cp_wbq.wait()
    cp_wbo.wait()
    w0_s[1] = _pack(wb_qkv[:, 2 * D:2 * D + 128])
    w0_s[2] = _pack(wb_o[:, 0:128])

    for l in range(2):
        src = xio_s if l == 0 else x_s
        a1_last_and_a2_first(src)
        lax.fori_loop(0, NTM - 1, functools.partial(a2b1_body, src), 0)
        b1_last_and_attn()
        attn_loop()
        if l == 0:
            a_reset()
            attn_tail_mid()
            lax.fori_loop(1, NTM - 1, b3a1_body, 0)
        else:
            attn_tail_final()
            for i in range(2 * QPS):
                cp_out(i).start()
            for i in range(2 * QPS, NTM - 1):
                b3out(i * TM, TM)
                cp_out(i).start()
            for h in range(2):
                b3out(S - TM + h * (TM // 2), TM // 2)
                cp_last(h).start()
    for i in range(NTM - 1):
        cp_out(i).wait()
    for h in range(2):
        cp_last(h).wait()


@jax.jit
def pallas_interleave_layers__linear_attn_block__mha_block__prompt_kernel(
    A_x: jax.Array,
    A_wqkv: jax.Array,
    A_wo: jax.Array,
    B_x: jax.Array,
    B_wqkv: jax.Array,
    B_wo: jax.Array,
):
    del B_x
    x = A_x.reshape(S, D)
    any_spec = pl.BlockSpec(memory_space=pl.ANY)
    out = pl.pallas_call(
        _kernel,
        out_shape=jax.ShapeDtypeStruct((S, D), BF16),
        in_specs=[any_spec] * 5,
        out_specs=any_spec,
        scratch_shapes=[
            pltpu.VMEM((S, D), BF16),
            pltpu.VMEM((S, D), F32),
            pltpu.VMEM((TM // 2, D), U32),
            pltpu.VMEM((D, 3 * D), BF16),
            pltpu.VMEM((D, D), BF16),
            pltpu.VMEM((D, 3 * D), BF16),
            pltpu.VMEM((D, D), BF16),
            pltpu.VMEM((S // 2, D), U32),
            pltpu.VMEM((G, 64, TM), U32),
            pltpu.VMEM((D // 2, S), U32),
            pltpu.VMEM((G, S // 2, 128), U32),
            pltpu.VMEM((D // 2, S), U32),
            pltpu.VMEM((G, 128, 128), F32),
            pltpu.VMEM((8, D), F32),
            pltpu.VMEM((G, 8, 128), U32),
            pltpu.VMEM((D // 2, D), U32),
            pltpu.VMEM((NV, S, TQ), F32),
            pltpu.VMEM((NV, 8, TQ), F32),
            pltpu.VMEM((HPG, DH, 8, TQ), F32),
            pltpu.VMEM((G, 128, NOFF, 128), F32),
            pltpu.VMEM((3, D // 2, 128), U32),
            pltpu.SMEM((1,), jnp.int32),
            pltpu.SemaphoreType.DMA((NTM + 1,)),
            pltpu.SemaphoreType.DMA((7,)),
        ],
        compiler_params=pltpu.CompilerParams(vmem_limit_bytes=128 * 1024 * 1024),
    )(x, A_wqkv, A_wo, B_wqkv, B_wo)
    return out.reshape(1, S, D)
```
